```python
import jax
import jax.numpy as jnp

def _softmax(x, axis=-1):
    return jax.nn.softmax(x, axis=axis)

def _gelu(x):
    return jax.nn.gelu(x, approximate=True)

def _silu(x):
    return jax.nn.silu(x)

def _sigmoid(x):
    return jax.nn.sigmoid(x)

def _layernorm(x, axis=-1, eps=1e-05):
    m = jnp.mean(x, axis=axis, keepdims=True)
    v = jnp.var(x, axis=axis, keepdims=True)
    return (x - m) / jnp.sqrt(v + eps)

def _scatter_add(tgt, idx, src, axis=0):
    return tgt.at[idx].add(src)

def _segment_sum(src, seg, n):
    return jax.ops.segment_sum(src, seg, n)

class _Rng:

    def __init__(self, key):
        self._k = key

    def _next(self):
        self._k, sub = jax.random.split(self._k)
        return sub

    def normal(self, shape):
        return jax.random.normal(self._next(), shape, dtype=jnp.bfloat16)

    def randint(self, lo, hi, shape):
        return jax.random.randint(self._next(), shape, lo, hi, dtype=jnp.int32)

    def uniform(self, shape, lo=0.0, hi=1.0):
        return jax.random.uniform(self._next(), shape, jnp.bfloat16, lo, hi)

    def permutation(self, n):
        return jax.random.permutation(self._next(), n)
kernel_name = 'gated_mix__memory_aug_recurrent_mem_tr__moe_arch_mod__prompt'

def setup_inputs():
    _rng = _Rng(jax.random.key(int.from_bytes(__import__("os").urandom(4), "little")))
    _w = lambda a: (lambda t: t.astype(jnp.bfloat16) if jnp.issubdtype(t.dtype, jnp.floating) else t)(jnp.asarray(a))

    def _A_setup():
        B, S, Dm = (1, 2048, 1024)
        H, Dh = (32, 128)
        M, seg = (8, 32)
        seg = min(seg, S)
        S = S // seg * seg
        return {'x': _w((lambda *s: _rng.normal(s) * 0.05)(B, S, Dm)), 'mem0': _w((lambda *s: _rng.normal(s) * 0.05)(B, M, Dm)), 'Wq': _w((lambda *s: _rng.normal(s) * 0.05)(Dm, H, Dh) * Dm ** (-0.5)), 'Wk': _w((lambda *s: _rng.normal(s) * 0.05)(Dm, H, Dh) * Dm ** (-0.5)), 'Wv': _w((lambda *s: _rng.normal(s) * 0.05)(Dm, H, Dh) * Dm ** (-0.5)), 'Wo': _w((lambda *s: _rng.normal(s) * 0.05)(H, Dh, Dm) * (H * Dh) ** (-0.5)), 'seg_len': seg}
    _A_in = _A_setup()

    def _B_setup():
        B, S, D, F, C = (1, 2048, 1024, 3584, 8)
        return {'x': _w((lambda *s: _rng.normal(s) * 0.05)(B, S, D)), 'w_r': _w((lambda *s: _rng.normal(s) * 0.05)(D)), 'w_gate': _w((lambda *s: _rng.normal(s) * 0.05)(D, F)), 'w_up': _w((lambda *s: _rng.normal(s) * 0.05)(D, F)), 'w_down': _w((lambda *s: _rng.normal(s) * 0.05)(F, D))}
    _B_in = _B_setup()
    return {'A_x': _A_in['x'], 'A_mem0': _A_in['mem0'], 'A_Wq': _A_in['Wq'], 'A_Wk': _A_in['Wk'], 'A_Wv': _A_in['Wv'], 'A_Wo': _A_in['Wo'], 'A_seg_len': _A_in['seg_len'], 'B_x': _B_in['x'], 'B_w_r': _B_in['w_r'], 'B_w_gate': _B_in['w_gate'], 'B_w_up': _B_in['w_up'], 'B_w_down': _B_in['w_down'], 'gate_w': _w((lambda *s: _rng.normal(s) * 0.05)(1024))}

def reference(A_x, A_mem0, A_Wq, A_Wk, A_Wv, A_Wo, A_seg_len, B_x, B_w_r, B_w_gate, B_w_up, B_w_down, gate_w):

    def _A_ref(x, mem0, Wq, Wk, Wv, Wo, seg_len):
        B, S, Dm = x.shape
        H, Dh = (Wq.shape[1], Wq.shape[2])
        M = mem0.shape[1]
        scale = Dh ** (-0.5)
        n_seg = S // seg_len
        L = M + seg_len
        idx = jnp.arange(L)
        mask = (idx[:, None] < M) | (idx[:, None] >= idx[None, :])
        mem = mem0
        outs = []
        for s in range(n_seg):
            xs = x[:, s * seg_len:(s + 1) * seg_len, :].copy()
            h = jnp.concatenate([mem, xs], axis=1)
            q = jnp.einsum('btd,dhe->bhte', h, Wq)
            k = jnp.einsum('btd,dhe->bhte', h, Wk)
            v = jnp.einsum('btd,dhe->bhte', h, Wv)
            scores = jnp.einsum('bhqe,bhke->bhqk', q, k) * scale
            scores = jnp.where(mask[None, None], scores, -1000000000.0)
            p = _softmax(scores, axis=-1)
            o = jnp.einsum('bhqk,bhke->bhqe', p, v)
            o = jnp.einsum('bhte,hed->btd', o, Wo)
            mem = o[:, :M, :].copy()
            outs.append(o[:, M:, :])
        return jnp.concatenate(outs, axis=1)

    def _B_ref(x, w_r, w_gate, w_up, w_down):
        B, S, D = x.shape
        C = 8
        r = x @ w_r
        idx = jnp.argsort(-r, axis=-1)[:, :C]
        idx_e = jnp.repeat(idx.reshape(B, C, 1), D, axis=2)
        x_sel = jnp.take_along_axis(x, idx_e, axis=1)
        g = _silu(x_sel @ w_gate)
        u = x_sel @ w_up
        y = g * u @ w_down
        r_sel = _sigmoid(jnp.take_along_axis(r, idx, axis=1))
        y = y * r_sel.reshape(B, C, 1)
        b_off = (jnp.arange(B) * S).reshape(B, 1)
        flat_idx = (idx + b_off).reshape(B * C)
        zero = (x * 0.0).reshape(B * S, D)
        upd = _scatter_add(zero, flat_idx, y.reshape(B * C, D), axis=0)
        return x + upd.reshape(B, S, D)
    x = A_x
    g = _sigmoid((x * gate_w).sum(-1, keepdims=True))
    a = _A_ref(x, A_mem0, A_Wq, A_Wk, A_Wv, A_Wo, A_seg_len)
    b = _B_ref(x, B_w_r, B_w_gate, B_w_up, B_w_down)
    return g * a + (1 - g) * b
```

```python
import functools
import math

import jax
import jax.numpy as jnp
from jax import lax
import jax.experimental.pallas as pl
import jax.experimental.pallas.tpu as pltpu

_F32 = jnp.float32
_BF16 = jnp.bfloat16
_LANES = 128
_TOPK = 8
_STEP_ROWS = 32
_GROUP = 4
_FFN_CHUNK = 4


def _dot(a, b):
    return jnp.dot(a, b, preferred_element_type=_F32)


def _dot_nt(a, b):
    return lax.dot_general(a, b, (((1,), (1,)), ((), ())), preferred_element_type=_F32)


def _kernel(
    x_hbm, mem0_ref, wq_hbm, wk_hbm, wv_hbm, wo_hbm, wr_ref, gw_ref,
    wg_hbm, wu_hbm, wd_hbm,
    out_hbm,
    x_sc, b_sc, w_sc, wo_sc, ring, wg_sc, wu_sc, wd_sc,
    w_sem, x_sem, wo_sem, ffn_sem, out_sem,
    *, seg,
):
    S, D = x_sc.shape
    M = mem0_ref.shape[0]
    H = w_sc.shape[0] * 2 // 3
    E = _LANES
    L = M + seg
    n_seg = S // seg
    ts = _STEP_ROWS - M
    r0 = S - n_seg * ts
    n_ring = ring.shape[1]
    n_pair = H // 2
    n_d = D // _LANES
    n_f = wg_sc.shape[0]
    scale = float(E) ** -0.5

    w_hbm = [w.bitcast(jnp.uint32) for w in (wq_hbm, wk_hbm, wv_hbm)]

    def w_copy(j, t):
        return pltpu.make_async_copy(
            w_hbm[t].at[:, :, j, :], w_sc.at[3 * j + t], w_sem.at[3 * j + t])

    x_head = pltpu.make_async_copy(x_hbm.at[pl.ds(0, r0)], x_sc.at[pl.ds(0, r0)], x_sem.at[0])
    x_tail = pltpu.make_async_copy(
        x_hbm.at[pl.ds(r0, S - r0)], x_sc.at[pl.ds(r0, S - r0)], x_sem.at[1])
    b_copy = pltpu.make_async_copy(x_hbm, b_sc, x_sem.at[2])

    def lane_block(n):
        return pl.ds(pl.multiple_of(n * _LANES, _LANES), _LANES)

    def wo_copy(n):
        return pltpu.make_async_copy(wo_hbm.at[:, lane_block(n)], wo_sc.at[n], wo_sem.at[0])

    def wg_copy(n):
        return pltpu.make_async_copy(wg_hbm.at[:, lane_block(n)], wg_sc.at[n], ffn_sem.at[0])

    def wu_copy(n):
        return pltpu.make_async_copy(wu_hbm.at[:, lane_block(n)], wu_sc.at[n], ffn_sem.at[1])

    def wd_copy(n):
        return pltpu.make_async_copy(wd_hbm.at[:, lane_block(n)], wd_sc.at[n], ffn_sem.at[2])

    def split_heads(j):
        for t in range(3):
            even = w_sc[3 * j + t, :, pl.ds(0, 8, stride=2), :]
            odd = w_sc[3 * j + t, :, pl.ds(1, 8, stride=2), :]
            w_sc[3 * j + t, :, 0:8, :] = (even & jnp.uint32(0xFFFF)) | (odd << 16)
            w_sc[3 * j + t, :, 8:16, :] = (even >> 16) | (odd & jnp.uint32(0xFFFF0000))

    def weight(j, p, t):
        w = w_sc[3 * j + t, :, 8 * p:8 * p + 8, :]
        return pltpu.bitcast(w.reshape(D // 2, E), _BF16)

    for t in range(3):
        w_copy(0, t).start()
    x_head.start()
    for j in (1, 2):
        for t in range(3):
            w_copy(j, t).start()
    x_tail.start()

    for t in range(3):
        w_copy(0, t).wait()
    split_heads(0)
    x_head.wait()

    def project(j):
        xs = x_sc[0:r0, :]
        for p in range(2):
            for t in range(3):
                ring[3 * (2 * j + p) + t, 0:r0, :] = _dot(xs, weight(j, p, t))

    n_early = n_pair // 2

    def phase1(j, carry):
        @pl.when(j + 3 < n_pair)
        def _():
            for t in range(3):
                w_copy(j + 3, t).start()

        @pl.when(j < n_early)
        def _():
            for i in range(n_d // n_early):
                wo_copy(j * (n_d // n_early) + i).start()

        @pl.when(j == n_early)
        def _():
            b_copy.start()

        for i in range(2):
            @pl.when(2 * j + i < n_f)
            def _():
                wg_copy(2 * j + i).start()
                wu_copy(2 * j + i).start()

        @pl.when(j >= n_pair - 1 - n_d)
        def _():
            wd_copy(j - (n_pair - 1 - n_d)).start()

        for t in range(3):
            w_copy(j + 1, t).wait()
        project(j)
        split_heads(j + 1)
        return carry

    lax.fori_loop(0, n_pair - 1, phase1, 0)
    x_tail.wait()
    project(n_pair - 1)

    wr = wr_ref[...].astype(_F32)
    gw = gw_ref[...].astype(_F32)
    lane = lax.broadcasted_iota(jnp.int32, (8, _LANES), 1)
    sub = lax.broadcasted_iota(jnp.int32, (8, _LANES), 0)
    n_slab = S // (8 * _LANES)
    scores, tokens = [], []
    for v in range(n_slab):
        acc = jnp.zeros((8, _LANES), _F32)
        for i in range(0, _LANES, 2):
            row = (v * _LANES + i) * 8
            r = jnp.sum(x_sc[row:row + 16, :].astype(_F32) * wr, axis=-1, keepdims=True)
            acc = jnp.where(lane == i, r[0:8], acc)
            acc = jnp.where(lane == i + 1, r[8:16], acc)
        acc = acc.astype(_BF16).astype(_F32)
        scores.append(jnp.where(acc != acc, -jnp.inf, acc))
        tokens.append(((v * _LANES + lane) * 8 + sub).astype(_F32))
    score = jnp.concatenate(scores, axis=0)
    token = jnp.concatenate(tokens, axis=0)

    picks = []
    row8 = lax.broadcasted_iota(jnp.int32, (_TOPK, 1), 0)
    row16 = lax.broadcasted_iota(jnp.int32, (16, 1), 0)
    r_sel = jnp.zeros((_TOPK, 1), _F32)
    x_sel = jnp.zeros((_TOPK, D), _F32)
    for c in range(_TOPK):
        best = jnp.max(jnp.max(score, axis=0, keepdims=True), axis=1, keepdims=True)
        first = jnp.where(score == best, token, float(S))
        first = jnp.min(jnp.min(first, axis=0, keepdims=True), axis=1, keepdims=True)
        taken = token == first
        score = jnp.where(taken, -jnp.inf, score)
        token = jnp.where(taken, float(S), token)
        idx = jnp.clip(first.astype(jnp.int32)[0, 0], 0, S - 1)
        base = pl.multiple_of((idx // 16) * 16, 16)
        hit = row16 == idx - base
        rows = x_sc[pl.ds(base, 16), :].astype(_F32)
        picked = jnp.sum(jnp.where(hit, rows, 0.0), axis=0, keepdims=True)
        x_sel = jnp.where(row8 == c, picked, x_sel)
        r_sel = jnp.where(row8 == c, best, r_sel)
        picks.append((base, hit))

    pltpu.make_async_copy(wg_sc, wg_sc, ffn_sem.at[0]).wait()
    pltpu.make_async_copy(wu_sc, wu_sc, ffn_sem.at[1]).wait()
    pltpu.make_async_copy(wd_sc, wd_sc, ffn_sem.at[2]).wait()
    b_copy.wait()
    pltpu.make_async_copy(wo_sc, wo_sc, wo_sem.at[0]).wait()
    hidden = []
    for n in range(n_f):
        gate = _dot(x_sel, wg_sc[n])
        hidden.append(gate * jax.nn.sigmoid(gate) * _dot(x_sel, wu_sc[n]))
    hidden = jnp.concatenate(hidden, axis=1).astype(_BF16).astype(_F32)
    y = jnp.concatenate([_dot(hidden, wd_sc[n]) for n in range(n_d)], axis=1)
    y = y * jax.nn.sigmoid(r_sel)
    for c, (base, hit) in enumerate(picks):
        rows = b_sc[pl.ds(base, 16), :].astype(_F32)
        b_sc[pl.ds(base, 16), :] = jnp.where(hit, rows + y[c:c + 1, :], rows).astype(_BF16)

    qi = lax.broadcasted_iota(jnp.int32, (L, L), 0)
    ki = lax.broadcasted_iota(jnp.int32, (L, L), 1)
    visible = (qi < M) | (ki >= seg) | (ki <= qi - M)
    n_grp = H // _GROUP

    def step(s, mem):
        src = pl.multiple_of(r0 + s * ts, 8)
        fresh = x_sc[pl.ds(src, ts), :].astype(_F32)
        lhs = jnp.concatenate([mem, fresh], axis=0).astype(_BF16)
        put = [pl.multiple_of(lax.rem(src + 8 * i, n_ring), 8) for i in range(ts // 8)]
        get = pl.multiple_of(lax.rem(s * seg, n_ring), seg)

        def proj(h, t):
            y = _dot(lhs, weight(h // 2, h % 2, t))
            for i in range(ts // 8):
                ring[3 * h + t, pl.ds(put[i], 8), :] = y[M + 8 * i:M + 8 * i + 8]
            tok = ring[3 * h + t, pl.ds(get, seg), :]
            if t == 0:
                return jnp.concatenate([y[:M], tok], axis=0)
            return jnp.concatenate([tok, y[:M]], axis=0).astype(_BF16)

        def probs(q, k):
            sc = jnp.where(visible, _dot_nt(q, k) * scale, -1e9)
            p = jnp.exp(sc - jnp.max(sc, axis=-1, keepdims=True))
            return p, jnp.sum(p, axis=-1, keepdims=True)

        def mix(p, v):
            return _dot(p[0], v) * pl.reciprocal(p[1], approx=False)

        acc = [None] * n_d

        def out_proj(g, o, blocks):
            rows = slice(g * _GROUP * E, (g + 1) * _GROUP * E)
            for n in blocks:
                y = _dot(o, wo_sc[n, rows, :])
                acc[n] = y if acc[n] is None else acc[n] + y

        p_prev = v_prev = o_prev = None
        for g in range(n_grp):
            heads = range(g * _GROUP, (g + 1) * _GROUP)
            q = [proj(h, 0) for h in heads]
            if g > 0:
                o_prev = jnp.concatenate(
                    [mix(p, v) for p, v in zip(p_prev, v_prev)], axis=1)
            k = [proj(h, 1) for h in heads]
            v = [proj(h, 2) for h in heads[:_GROUP // 2]]
            p_prev = [probs(a, b) for a, b in zip(q, k)]
            v_prev = v + [proj(h, 2) for h in heads[_GROUP // 2:]]
            if 0 < g < n_grp - 1:
                out_proj(g - 1, o_prev, range(n_d))
        out_proj(n_grp - 2, o_prev, range(n_d // 2))
        o_last = jnp.concatenate([mix(p, v) for p, v in zip(p_prev, v_prev)], axis=1)
        out_proj(n_grp - 2, o_prev, range(n_d // 2, n_d))
        out_proj(n_grp - 1, o_last, range(n_d))
        res = jnp.concatenate(acc, axis=1)

        row = pl.ds(pl.multiple_of(s * seg, seg), seg)
        gate = jax.nn.sigmoid(
            jnp.sum(x_sc[row, :].astype(_F32) * gw, axis=-1, keepdims=True))
        b_sc[row, :] = (gate * res[M:] + (1.0 - gate) * b_sc[row, :].astype(_F32)).astype(_BF16)
        pltpu.make_async_copy(b_sc.at[row], out_hbm.at[row], out_sem.at[0]).start()
        return res[:M]

    lax.fori_loop(0, n_seg, step, mem0_ref[...].astype(_F32))
    pltpu.make_async_copy(b_sc, out_hbm, out_sem.at[0]).wait()


@functools.partial(jax.jit, static_argnames=("A_seg_len",))
def pallas_gated_mix__memory_aug_recurrent_mem_tr__moe_arch_mod__prompt_kernel(
    A_x: jax.Array,
    A_mem0: jax.Array,
    A_Wq: jax.Array,
    A_Wk: jax.Array,
    A_Wv: jax.Array,
    A_Wo: jax.Array,
    A_seg_len: int,
    B_x: jax.Array,
    B_w_r: jax.Array,
    B_w_gate: jax.Array,
    B_w_up: jax.Array,
    B_w_down: jax.Array,
    gate_w: jax.Array,
):
    del B_x
    B, S, D = A_x.shape
    M = A_mem0.shape[1]
    H, E = A_Wq.shape[1:]
    F = B_w_gate.shape[1]
    seg = int(A_seg_len)
    assert B == 1 and E == _LANES and M == 8 and seg == _STEP_ROWS and S % seg == 0
    n_ring = S - (S // seg) * (_STEP_ROWS - M) + seg

    hbm = pl.BlockSpec(memory_space=pl.ANY)
    vmem = pl.BlockSpec(memory_space=pltpu.VMEM)
    slabs = lambda w: w.reshape(D // 16, 16, H, E)
    out = pl.pallas_call(
        functools.partial(_kernel, seg=seg),
        out_shape=jax.ShapeDtypeStruct((S, D), A_x.dtype),
        in_specs=[hbm, vmem, hbm, hbm, hbm, hbm, vmem, vmem, hbm, hbm, hbm],
        out_specs=hbm,
        scratch_shapes=[
            pltpu.VMEM((S, D), _BF16),
            pltpu.VMEM((S, D), _BF16),
            pltpu.VMEM((3 * H // 2, D // 16, 16, E), jnp.uint32),
            pltpu.VMEM((D // _LANES, H * E, _LANES), _BF16),
            pltpu.VMEM((3 * H, n_ring, E), _F32),
            pltpu.VMEM((F // _LANES, D, _LANES), _BF16),
            pltpu.VMEM((F // _LANES, D, _LANES), _BF16),
            pltpu.VMEM((D // _LANES, F, _LANES), _BF16),
            pltpu.SemaphoreType.DMA((3 * H // 2,)),
            pltpu.SemaphoreType.DMA((3,)),
            pltpu.SemaphoreType.DMA((1,)),
            pltpu.SemaphoreType.DMA((3,)),
            pltpu.SemaphoreType.DMA((1,)),
        ],
        compiler_params=pltpu.CompilerParams(vmem_limit_bytes=112 * 1024 * 1024),
    )(
        A_x.reshape(S, D), A_mem0.reshape(M, D),
        slabs(A_Wq), slabs(A_Wk), slabs(A_Wv), A_Wo.reshape(H * E, D),
        B_w_r.reshape(1, D), gate_w.reshape(1, D),
        B_w_gate, B_w_up, B_w_down,
    )
    return out.reshape(B, S, D)
```

```python
import functools

import jax
import jax.numpy as jnp
from jax import lax
import jax.experimental.pallas as pl
import jax.experimental.pallas.tpu as pltpu

_F32 = jnp.float32
_BF16 = jnp.bfloat16
_U32 = jnp.uint32
_LANES = 128
_TOPK = 8
_STEP_ROWS = 32
_GROUP = 4
_UNROLL = 2
_EARLY = 3


def _dot(a, b):
    return jnp.dot(a, b, preferred_element_type=_F32)


def _kernel(
    x_hbm, mem0_ref, wq_hbm, wk_hbm, wv_hbm, wo_hbm, wr_ref, gw_ref,
    wg_hbm, wu_hbm, wd_hbm,
    out_hbm,
    x_sc, o_sc, a_sc, y_sc, w_sc, wo_sc, ring, wg_sc, wu_sc, wd_sc,
    w_sem, x_sem, wo_sem, ffn_sem, out_sem,
    *, seg,
):
    S, D = x_sc.shape
    M = mem0_ref.shape[0]
    H = w_sc.shape[0] * 2 // 3
    E = _LANES
    L = M + seg
    n_seg = S // seg
    ts = _STEP_ROWS - M
    r0 = S - n_seg * ts
    n_ring = ring.shape[1]
    n_pair = H // 2
    n_d = D // _LANES
    n_f = wg_sc.shape[0]
    scale = float(E) ** -0.5

    w_hbm = [w.bitcast(_U32) for w in (wq_hbm, wk_hbm, wv_hbm)]
    wo_hbm, wg_hbm, wu_hbm, wd_hbm = [
        w.bitcast(_U32) for w in (wo_hbm, wg_hbm, wu_hbm, wd_hbm)]

    def w_copy(j, t):
        j, t = j + t // 3, t % 3
        return pltpu.make_async_copy(
            w_hbm[t].at[:, :, j, :], w_sc.at[3 * j + t],
            w_sem.at[(3 * j + t) & (w_sem.shape[0] - 1)])

    def x_copy(i):
        rows = pl.ds(pl.multiple_of(i * r0, r0), r0)
        return pltpu.make_async_copy(x_hbm.at[rows], x_sc.at[rows], x_sem.at[0])

    def lane_block(n):
        return pl.ds(pl.multiple_of(n * _LANES, _LANES), _LANES)

    def wo_copy(n):
        return pltpu.make_async_copy(wo_hbm.at[:, lane_block(n)], wo_sc.at[n], wo_sem.at[0])

    def ffn_copies(n):
        sem = ffn_sem.at[n & 1]
        rows = pl.ds(pl.multiple_of(n * (_LANES // 2), _LANES // 2), _LANES // 2)
        return [pltpu.make_async_copy(wg_hbm.at[:, lane_block(n)], wg_sc.at[n], sem),
                pltpu.make_async_copy(wu_hbm.at[:, lane_block(n)], wu_sc.at[n], sem),
                pltpu.make_async_copy(wd_hbm.at[rows], wd_sc.at[n], sem)]

    def out_copy(first, count):
        rows = pl.ds(pl.multiple_of(first * seg, seg), count * seg)
        return pltpu.make_async_copy(o_sc.at[rows], out_hbm.at[rows], out_sem.at[0])

    def split_heads(j, t):
        u = 3 * j + t
        for c in range(0, D // 16, 8):
            even = w_sc[u, c:c + 8, pl.ds(0, 8, stride=2), :]
            odd = w_sc[u, c:c + 8, pl.ds(1, 8, stride=2), :]
            w_sc[u, c:c + 8, 0:8, :] = (even & _U32(0xFFFF)) | (odd << 16)
            w_sc[u, c:c + 8, 8:16, :] = (even >> 16) | (odd & _U32(0xFFFF0000))

    def weight(j, p, t, lo=0, hi=D):
        w = w_sc[3 * j + t, lo // 16:hi // 16, 8 * p:8 * p + 8, :]
        return pltpu.bitcast(w.reshape((hi - lo) // 2, E), _BF16)

    x_copy(0).start()
    w_copy(0, 0).start()
    o_sc[...] = jnp.zeros(o_sc.shape, _BF16)
    a_sc[...] = jnp.zeros(a_sc.shape, _F32)
    y_sc[...] = jnp.zeros(y_sc.shape, _F32)
    w_copy(0, 0).wait()
    w_copy(0, 1).start()
    split_heads(0, 0)
    x_copy(0).wait()
    w_copy(0, 2).start()

    wr = wr_ref[...].astype(_F32).reshape(1, D)
    gw = gw_ref[...].astype(_F32).reshape(1, D)

    n_tok = S // n_pair
    slot = (lax.broadcasted_iota(jnp.int32, (S // _LANES, _LANES), 0) // 8 * _LANES
            + lax.broadcasted_iota(jnp.int32, (S // _LANES, _LANES), 1))

    def project(j, score, overlap):
        xs = x_sc[0:r0, :]
        for t in range(3):
            for p in range(2):
                ring[3 * (2 * j + p) + t, 0:r0, :] = _dot(xs, weight(j, p, t))
                if p == 0:
                    overlap(j, t)
        for i in range(0, n_tok, 16):
            rows = pl.ds(pl.multiple_of(j * n_tok + i, 16), 16)
            r = jnp.sum(x_sc[rows, :].astype(_F32) * wr, axis=-1, keepdims=True)
            for c in range(2):
                part = jnp.concatenate([r[8 * c:8 * c + 8]] * (S // _LANES // 8), axis=0)
                score = jnp.where(slot == (j * n_tok + i) // 8 + c, part, score)
        return score

    per_x = r0 // n_tok

    def overlap_first(j, t):
        w_copy(j, t + 1).wait()
        for u in range(t + 3, t + 4 if t < 2 else 7):
            w_copy(j, u).start()
        split_heads(j, t + 1)

    def overlap_middle(j, t):
        @pl.when(3 * j + t + 4 < 3 * n_pair)
        def _():
            w_copy(j, t + 4).start()

        if t == 1:
            @pl.when(jnp.logical_and((j & (per_x - 1)) == 1, j < n_pair - per_x))
            def _():
                x_copy(j // per_x + 1).start()

        if t == 2:
            n = j - (j + per_x - 1) // per_x - 1

            @pl.when(jnp.logical_and((j & (per_x - 1)) != 1, n < n_d))
            def _():
                wo_copy(n).start()

        split_heads(j, t + 1)

    def overlap_last(j, t):
        if t == 0:
            for cp in ffn_copies(0):
                cp.start()
        if t < 2:
            split_heads(j, t + 1)

    def phase1(j, score):
        for t in range(1, 4):
            w_copy(j, t).wait()

        @pl.when((j & (per_x - 1)) == 0)
        def _():
            x_copy(j // per_x).wait()

        return project(j, score, overlap_middle)

    score = project(0, jnp.zeros((S // _LANES, _LANES), _F32), overlap_first)
    score = lax.fori_loop(1, n_pair - 1, phase1, score)
    for t in range(1, 3):
        w_copy(n_pair - 1, t).wait()
    score = project(n_pair - 1, score, overlap_last)

    score = score.astype(_BF16).astype(_F32)
    score = jnp.where(score != score, -jnp.inf, score)
    token = (slot * 8 + lax.broadcasted_iota(jnp.int32, slot.shape, 0) % 8).astype(_F32)
    picks = []
    row8 = lax.broadcasted_iota(jnp.int32, (_TOPK, 1), 0)
    row16 = lax.broadcasted_iota(jnp.int32, (16, 1), 0)
    r_sel = jnp.zeros((_TOPK, 1), _F32)
    x_sel = jnp.zeros((_TOPK, D), _F32)
    for c in range(_TOPK):
        best = jnp.max(jnp.max(score, axis=0, keepdims=True), axis=1, keepdims=True)
        first = jnp.where(score == best, token, float(S))
        first = jnp.min(jnp.min(first, axis=0, keepdims=True), axis=1, keepdims=True)
        taken = token == first
        score = jnp.where(taken, -jnp.inf, score)
        token = jnp.where(taken, float(S), token)
        idx = jnp.clip(first.astype(jnp.int32)[0, 0], 0, S - 1)
        base = pl.multiple_of((idx // 16) * 16, 16)
        rows = x_sc[pl.ds(base, 16), :].astype(_F32)
        picked = jnp.sum(jnp.where(row16 == idx - base, rows, 0.0), axis=0, keepdims=True)
        x_sel = jnp.where(row8 == c, picked, x_sel)
        r_sel = jnp.where(row8 == c, best, r_sel)
        picks.append((base, idx - base))
    o_sc[S:, :] = jnp.concatenate([x_sel, x_sel], axis=0).astype(_BF16)
    pltpu.make_async_copy(wo_sc, wo_sc, wo_sem.at[0]).wait()

    qi = lax.broadcasted_iota(jnp.int32, (L, L), 0)
    ki = lax.broadcasted_iota(jnp.int32, (L, L), 1)
    visible = (qi < M) | (ki >= seg) | (ki <= qi - M)
    n_grp = H // _GROUP

    def gate_of(x):
        return jax.nn.sigmoid(jnp.sum(x * gw, axis=-1, keepdims=True))

    y_scale = jax.nn.sigmoid(r_sel) * (1.0 - gate_of(x_sel))

    def emit(s, a, keep=None):
        row = pl.ds(pl.multiple_of(s * seg, seg), seg)
        x = x_sc[row, :].astype(_F32)
        gate = gate_of(x)
        mixed = gate * a + (1.0 - gate) * x
        if keep is not None:
            mixed = jnp.where(keep, mixed, 0.0)
        o_sc[row, :] = (o_sc[row, :].astype(_F32) + mixed).astype(_BF16)

    def ffn_block(n, live):
        gate = up = None
        for c in range(2):
            cols = slice(c * D // 2, (c + 1) * D // 2)
            rows = slice(c * D // 4, (c + 1) * D // 4)
            z = _dot(o_sc[S:, cols].astype(_F32)[:_TOPK], pltpu.bitcast(wg_sc[n, rows, :], _BF16))
            gate = z if c == 0 else z + gate
            yield
            z = _dot(o_sc[S:, cols].astype(_F32)[:_TOPK], pltpu.bitcast(wu_sc[n, rows, :], _BF16))
            up = z if c == 0 else z + up
            yield
        hidden = jnp.where(live, gate * jax.nn.sigmoid(gate) * up, 0.0)
        for c in range(2):
            cols = slice(c * D // 2, (c + 1) * D // 2)
            y_sc[:, cols] += _dot(hidden, pltpu.bitcast(wd_sc[n, :, cols], _BF16))
            yield

    def step(s, mem, ffn, n_early):
        src = pl.multiple_of(r0 + s * ts, 8)
        fresh = x_sc[pl.ds(src, ts), :].astype(_F32)
        lhs = jnp.concatenate([mem, fresh], axis=0).astype(_BF16)
        put = [pl.multiple_of(lax.rem(src + 8 * i, n_ring), 8) for i in range(ts // 8)]
        get = pl.multiple_of(lax.rem(s * seg, n_ring), seg)
        early = {(h, 0): _dot(lhs[:, :D // 2], weight(h // 2, h % 2, 0, 0, D // 2))
                 for h in range(n_early)}

        def proj(h, t):
            if (h, t) in early:
                y = _dot(lhs[:, D // 2:], weight(h // 2, h % 2, t, D // 2, D)) + early[h, t]
            else:
                y = _dot(lhs, weight(h // 2, h % 2, t))
            for i in range(ts // 8):
                ring[3 * h + t, pl.ds(put[i], 8), :] = y[M + 8 * i:M + 8 * i + 8]
            tok = ring[3 * h + t, pl.ds(get, seg), :]
            if t == 0:
                return jnp.concatenate([y[:M], tok], axis=0)
            return jnp.concatenate([tok, y[:M]], axis=0).astype(_BF16)

        def probs(q, k):
            sc = lax.dot_general(q, k, (((1,), (1,)), ((), ())), preferred_element_type=_F32)
            sc = jnp.where(visible, sc * scale, -1e9)
            p = jnp.exp(sc - jnp.max(sc, axis=-1, keepdims=True))
            return p, jnp.sum(p, axis=-1, keepdims=True)

        def mix(ps, vs):
            return jnp.concatenate(
                [_dot(p, v) * pl.reciprocal(total, approx=True)
                 for (p, total), v in zip(ps, vs)], axis=1)

        acc = [None] * n_d

        def out_proj(g, blocks):
            rows = slice(g * _GROUP * E // 2, (g + 1) * _GROUP * E // 2)
            for n in blocks:
                y = _dot(o[g], pltpu.bitcast(wo_sc[n, rows, :], _BF16))
                acc[n] = y if acc[n] is None else y + acc[n]
                if n == n_d // 2 and g % 2 == 1 and g < n_grp - 2:
                    next(ffn, None)

        o = {}
        p_prev = v_prev = None
        for g in range(n_grp):
            heads = range(g * _GROUP, (g + 1) * _GROUP)
            q = [proj(h, 0) for h in heads]
            k = [proj(h, 1) for h in heads]
            if g > 0:
                o[g - 1] = mix(p_prev, v_prev)
            v_prev = [proj(h, 2) for h in heads]
            p_prev = [probs(a, b) for a, b in zip(q, k)]
            if g > 1:
                out_proj(g - 2, range(n_d))
        out_proj(n_grp - 2, range(n_d // 4))
        o[n_grp - 1] = mix(p_prev, v_prev)
        out_proj(n_grp - 2, range(n_d // 4, n_d))
        out_proj(n_grp - 1, range(n_d))
        res = jnp.concatenate(acc, axis=1)
        return res[:M], res[M:]

    def steps(i, mem):
        @pl.when(i < n_f)
        def _():
            for cp in ffn_copies(i):
                cp.wait()

        @pl.when(i + 1 < n_f)
        def _():
            for cp in ffn_copies(i + 1):
                cp.start()

        @pl.when(i == n_f)
        def _():
            y = y_sc[...] * y_scale
            for c, (base, off) in enumerate(picks):
                rows = o_sc[pl.ds(base, 16), :].astype(_F32)
                rows = jnp.where(row16 == off, rows + y[c:c + 1, :], rows)
                o_sc[pl.ds(base, 16), :] = rows.astype(_BF16)
            out_copy(0, _UNROLL * n_f - 1).start()

        ffn = ffn_block(jnp.minimum(i, n_f - 1), i < n_f)
        emit(jnp.maximum(_UNROLL * i - 1, 0), a_sc[...], i > 0)
        mem, a = step(_UNROLL * i, mem, ffn, 0)
        emit(_UNROLL * i, a)
        mem, a = step(_UNROLL * i + 1, mem, ffn, _EARLY)
        for _ in ffn:
            pass
        a_sc[...] = a

        @pl.when(i >= n_f)
        def _():
            out_copy(_UNROLL * i - 1, _UNROLL).start()

        return mem

    lax.fori_loop(0, n_seg // _UNROLL, steps, mem0_ref[...].astype(_F32))
    emit(n_seg - 1, a_sc[...])
    out_copy(n_seg - 1, 1).start()
    out_copy(0, n_seg).wait()


@functools.partial(jax.jit, static_argnames=("A_seg_len",))
def pallas_gated_mix__memory_aug_recurrent_mem_tr__moe_arch_mod__prompt_kernel(
    A_x: jax.Array,
    A_mem0: jax.Array,
    A_Wq: jax.Array,
    A_Wk: jax.Array,
    A_Wv: jax.Array,
    A_Wo: jax.Array,
    A_seg_len: int,
    B_x: jax.Array,
    B_w_r: jax.Array,
    B_w_gate: jax.Array,
    B_w_up: jax.Array,
    B_w_down: jax.Array,
    gate_w: jax.Array,
):
    del B_x
    B, S, D = A_x.shape
    M = A_mem0.shape[1]
    H, E = A_Wq.shape[1:]
    F = B_w_gate.shape[1]
    seg = int(A_seg_len)
    assert (B, S, D, M, H, E, seg) == (1, 2048, 1024, 8, 32, _LANES, _STEP_ROWS)
    assert F % _LANES == 0 and F // _LANES < S // seg // _UNROLL
    n_ring = S - (S // seg) * (_STEP_ROWS - M) + seg

    hbm = pl.BlockSpec(memory_space=pl.ANY)
    vmem = pl.BlockSpec(memory_space=pltpu.VMEM)
    slabs = lambda w: w.reshape(D // 16, 16, H, E)
    out = pl.pallas_call(
        functools.partial(_kernel, seg=seg),
        out_shape=jax.ShapeDtypeStruct((S, D), A_x.dtype),
        in_specs=[hbm, vmem, hbm, hbm, hbm, hbm, vmem, vmem, hbm, hbm, hbm],
        out_specs=hbm,
        scratch_shapes=[
            pltpu.VMEM((S, D), _BF16),
            pltpu.VMEM((S + 2 * _TOPK, D), _BF16),
            pltpu.VMEM((seg, D), _F32),
            pltpu.VMEM((_TOPK, D), _F32),
            pltpu.VMEM((3 * H // 2, D // 16, 16, E), _U32),
            pltpu.VMEM((D // _LANES, H * E // 2, _LANES), _U32),
            pltpu.VMEM((3 * H, n_ring, E), _F32),
            pltpu.VMEM((F // _LANES, D // 2, _LANES), _U32),
            pltpu.VMEM((F // _LANES, D // 2, _LANES), _U32),
            pltpu.VMEM((F // _LANES, _LANES // 2, D), _U32),
            pltpu.SemaphoreType.DMA((8,)),
            pltpu.SemaphoreType.DMA((1,)),
            pltpu.SemaphoreType.DMA((1,)),
            pltpu.SemaphoreType.DMA((2,)),
            pltpu.SemaphoreType.DMA((1,)),
        ],
        compiler_params=pltpu.CompilerParams(
            vmem_limit_bytes=112 * 1024 * 1024, disable_bounds_checks=True),
    )(
        A_x.reshape(S, D), A_mem0.reshape(M, D),
        slabs(A_Wq), slabs(A_Wk), slabs(A_Wv), A_Wo.reshape(H * E, D),
        B_w_r, gate_w, B_w_gate, B_w_up, B_w_down,
    )
    return out.reshape(B, S, D)
```

```python
import functools

import jax
import jax.numpy as jnp
from jax import lax
import jax.experimental.pallas as pl
import jax.experimental.pallas.tpu as pltpu

_F32 = jnp.float32
_BF16 = jnp.bfloat16
_U32 = jnp.uint32
_LANES = 128
_TOPK = 8
_STEP_ROWS = 32
_GROUP = 4
_UNROLL = 2
_EARLY = 3
_PIECE = 32
_MASKED = -1e9
_MIX_AT = 7
_FFN_AT = 3
_FFN_STAGES = (2, 3, 4)
_EMIT_BY = 6

_PLAN = ((2, ((1, 0), (3, 0))), (3, ((2, 0), (0, 0))), (4, ((1, 1), (0, -1))),
         (1, ((2, 1), (3, -1))), (0, ((0, 1), (3, 1))), (5, ((3, 1),)), (6, ((0, 1),)))
_RHS_SLOT = (0, None, 1, 2, None, 3, 4)


def _lhs_terms(a11, a12, a21, a22):
    return a11 + a22, a21 + a22, a11, a22, a11 + a12, a21 - a11, a12 - a22


def _rhs_terms(b11, b12, b21, b22):
    return b11 + b22, b12 - b22, b21 - b11, b11 + b12, b21 + b22


def _dot(a, b):
    return jnp.dot(a, b, preferred_element_type=_F32)


def _recip(x):
    r = pl.reciprocal(x, approx=True)
    return r * (2.0 - x * r)


def _kernel(
    x_hbm, mem0_hbm, wq_hbm, wk_hbm, wv_hbm, wo_hbm, wr_hbm, gw_hbm,
    wg_hbm, wu_hbm, wd_hbm,
    out_hbm,
    x_sc, o_sc, a_sc, y_sc, w_sc, wo_sc, ring, wg_sc, wu_sc, wd_sc,
    mem0_sc, wr_sc, gw_sc, xa_sc, wb_sc,
    w_sem, x_sem, wo_sem, ffn_sem, out_sem,
    *, seg,
):
    S, D = x_sc.shape
    M = mem0_sc.shape[0]
    H = w_sc.shape[0] * 2 // 3
    E = _LANES
    L = M + seg
    n_seg = S // seg
    ts = _STEP_ROWS - M
    r0 = S - n_seg * ts
    hr, hd = r0 // 2, D // 2
    n_ring = r0 + seg
    spare = slice(n_ring, n_ring + 8)
    n_pair = H // 2
    n_d = D // _LANES
    n_f = wg_hbm.shape[1] // _LANES
    scale = float(E) ** -0.5 * 1.4426950408889634

    w_hbm = [w.bitcast(_U32) for w in (wq_hbm, wk_hbm, wv_hbm)]
    wo_hbm, wg_hbm, wu_hbm, wd_hbm = [
        w.bitcast(_U32) for w in (wo_hbm, wg_hbm, wu_hbm, wd_hbm)]

    def w_copy(j, t):
        j, t = j + t // 3, t % 3
        return pltpu.make_async_copy(
            w_hbm[t].at[:, :, j, :], w_sc.at[3 * j + t],
            w_sem.at[(3 * j + t) & (w_sem.shape[0] - 1)])

    def x_copy(i):
        rows = pl.ds(pl.multiple_of(i * r0, r0), r0)
        return pltpu.make_async_copy(x_hbm.at[rows], x_sc.at[rows], x_sem.at[0])

    def lane_block(n):
        return pl.ds(pl.multiple_of(n * _LANES, _LANES), _LANES)

    def wo_copy(n):
        return pltpu.make_async_copy(wo_hbm.at[:, lane_block(n)], wo_sc.at[n], wo_sem.at[0])

    def ffn_copies(n):
        sem = ffn_sem.at[n & 1]
        rows = pl.ds(pl.multiple_of(n * (_LANES // 2), _LANES // 2), _LANES // 2)
        return [pltpu.make_async_copy(wg_hbm.at[:, lane_block(n)], wg_sc.at[n & 1], sem),
                pltpu.make_async_copy(wu_hbm.at[:, lane_block(n)], wu_sc.at[n & 1], sem),
                pltpu.make_async_copy(wd_hbm.at[rows], wd_sc.at[n & 1], sem)]

    def out_copy(first, count):
        rows = pl.ds(pl.multiple_of(first * seg, seg), count * seg)
        return pltpu.make_async_copy(o_sc.at[rows], out_hbm.at[rows], out_sem.at[0])

    def split_heads(j, t):
        u = 3 * j + t
        for c in range(hd // 16):
            hi = pltpu.bitcast(ring[2, spare, :], _U32)
            lo = hi >> 16
            blocks = []
            for slab in (c, c + hd // 16):
                even = w_sc[u, slab, pl.ds(0, 8, stride=2), :]
                odd = w_sc[u, slab, pl.ds(1, 8, stride=2), :]
                pair = (even & lo) | (odd << 16), (even >> 16) | (odd & hi)
                for p in range(2):
                    w_sc[u, slab, 8 * p:8 * p + 8, :] = pair[p]
                    blocks.append(pltpu.bitcast(pair[p], _BF16).astype(_F32))
            for i, z in enumerate(_rhs_terms(*blocks)):
                wb_sc[t % 3, i, 8 * c:8 * c + 8, :] = pltpu.bitcast(z.astype(_BF16), _U32)
            yield

    def weight(j, p, t, lo=0, hi=D):
        w = w_sc[3 * j + t, lo // 16:hi // 16, 8 * p:8 * p + 8, :]
        return pltpu.bitcast(w.reshape((hi - lo) // 2, E), _BF16)

    x_copy(0).start()
    w_copy(0, 0).start()
    small = [pltpu.make_async_copy(a, b, wo_sem.at[0])
             for a, b in ((mem0_hbm, mem0_sc), (wr_hbm, wr_sc), (gw_hbm, gw_sc))]
    for cp in small:
        cp.start()
    o_sc[...] = jnp.zeros(o_sc.shape, _BF16)
    a_sc[...] = jnp.zeros(a_sc.shape, _F32)
    y_sc[...] = jnp.zeros(y_sc.shape, _F32)
    ring[2, spare, :] = pltpu.bitcast(jnp.full((8, E), 0xFFFF0000, _U32), _F32)
    for cp in small:
        cp.wait()
    w_copy(0, 0).wait()
    w_copy(0, 1).start()
    for _ in split_heads(0, 0):
        pass
    x_copy(0).wait()
    w_copy(0, 2).start()
    for i in range(0, hr, 16):
        terms = _lhs_terms(*[x_sc[r + i:r + i + 16, c:c + hd].astype(_F32)
                             for r in (0, hr) for c in (0, hd)])
        for k, z in enumerate(terms):
            xa_sc[k, i // 2:i // 2 + 8, :] = pltpu.bitcast(z.astype(_BF16), _U32)

    wr = wr_sc[...].astype(_F32).reshape(1, D)
    gw = gw_sc[...].astype(_F32).reshape(1, D)

    n_tok = S // n_pair
    slot = (lax.broadcasted_iota(jnp.int32, (S // _LANES, _LANES), 0) // 8 * _LANES
            + lax.broadcasted_iota(jnp.int32, (S // _LANES, _LANES), 1))

    def route(score, row):
        r = jnp.sum(x_sc[pl.ds(pl.multiple_of(row, 16), 16), :].astype(_F32) * wr,
                    axis=-1, keepdims=True)
        for c in range(2):
            piece = jnp.concatenate([r[8 * c:8 * c + 8]] * (S // _LANES // 8), axis=0)
            score = jnp.where(slot == row // 8 + c, piece, score)
        return score

    def project(j, score, overlap):
        for t in range(3):
            side = overlap(j, t)
            for c, (k, outs) in enumerate(_PLAN):
                if k == 1:
                    w = weight(j, 0, t, 0, hd)
                elif k == 4:
                    w = weight(j, 1, t, hd, D)
                else:
                    w = pltpu.bitcast(wb_sc[t, _RHS_SLOT[k]], _BF16)
                m = _dot(pltpu.bitcast(xa_sc[k], _BF16), w)
                for r in range(0, hr, _PIECE):
                    for block, sign in outs:
                        row = block // 2 * hr + r
                        dst = (3 * (2 * j + block % 2) + t, slice(row, row + _PIECE))
                        z = m[r:r + _PIECE]
                        ring[dst] = z if sign == 0 else ring[dst] + z if sign > 0 else ring[dst] - z
                    if c >= 1:
                        next(side, None)
                if c >= 4:
                    ring[0, spare, :] = score[:8]
                    part = 16 * (3 * t + c - 4)
                    if part < n_tok:
                        score = route(score, j * n_tok + part)
            for _ in side:
                pass
        return score

    per_x = r0 // n_tok

    def overlap_first(j, t):
        for _ in range(hr // _PIECE):
            yield
        w_copy(j, t + 1).wait()
        for u in ((3, 4), (5, 6), (7,))[t]:
            w_copy(j, u).start()
        yield from split_heads(j, t + 1)

    def overlap_last(j, t):
        if t < 2:
            yield from split_heads(j, t + 1)

    def phase1(j, score):
        for t in range(1, 4):
            w_copy(j, t).wait()

        @pl.when((j & (per_x - 1)) == 0)
        def _():
            x_copy(j // per_x).wait()

        score = project(j, score, lambda j, t: split_heads(j, t + 1))

        for u in range(7, 10):
            @pl.when(3 * j + u < 3 * n_pair)
            def _():
                w_copy(j, u).start()

        @pl.when(jnp.logical_and((j & (per_x - 1)) == 1, j < n_pair - per_x))
        def _():
            x_copy(j // per_x + 1).start()

        n = j - (j + per_x - 1) // per_x - 1

        @pl.when(jnp.logical_and((j & (per_x - 1)) != 1, n < n_d))
        def _():
            wo_copy(n).start()

        return score

    score = project(0, jnp.zeros((S // _LANES, _LANES), _F32), overlap_first)
    for u in (8, 9):
        w_copy(0, u).start()
    score = lax.fori_loop(1, n_pair - 1, phase1, score)
    for cp in ffn_copies(0):
        cp.start()
    for t in range(1, 3):
        w_copy(n_pair - 1, t).wait()
    score = project(n_pair - 1, score, overlap_last)

    score = score.astype(_BF16).astype(_F32)
    score = jnp.where(score != score, -jnp.inf, score)
    token = (slot * 8 + lax.broadcasted_iota(jnp.int32, slot.shape, 0) % 8).astype(_F32)
    picks = []
    row8 = lax.broadcasted_iota(jnp.int32, (8, 1), 0)
    row16 = lax.broadcasted_iota(jnp.int32, (16, 1), 0)
    r_sel = jnp.zeros((_TOPK, 1), _F32)
    x_sel = jnp.zeros((_TOPK, D), _F32)
    for c in range(_TOPK):
        best = jnp.max(jnp.max(score, axis=0, keepdims=True), axis=1, keepdims=True)
        first = jnp.where(score == best, token, float(S))
        first = jnp.min(jnp.min(first, axis=0, keepdims=True), axis=1, keepdims=True)
        taken = token == first
        score = jnp.where(taken, -jnp.inf, score)
        token = jnp.where(taken, float(S), token)
        idx = jnp.clip(first.astype(jnp.int32)[0, 0], 0, S - 1)
        base = pl.multiple_of((idx // 16) * 16, 16)
        rows = x_sc[pl.ds(base, 16), :].astype(_F32)
        picked = jnp.sum(jnp.where(row16 == idx - base, rows, 0.0), axis=0, keepdims=True)
        x_sel = jnp.where(row8 == c, picked, x_sel)
        r_sel = jnp.where(row8 == c, best, r_sel)
        picks.append((base, idx - base))
    o_sc[S:, :] = jnp.concatenate([x_sel, x_sel], axis=0).astype(_BF16)
    pltpu.make_async_copy(wo_sc, wo_sc, wo_sem.at[0]).wait()

    n_grp = H // _GROUP

    def mask_bias(skip):
        qi = lax.broadcasted_iota(jnp.int32, (L - skip, L), 0)
        ki = lax.broadcasted_iota(jnp.int32, (L - skip, L), 1)
        return jnp.where((qi < M) | (ki >= seg) | (ki <= qi - M + skip), 0.0, _MASKED)

    bias = {skip: mask_bias(skip) for skip in (0, 8)}
    edge = {j: jnp.where(row8 >= j, 0.0, _MASKED) for j in range(1, 8)}

    def gate_of(x):
        return jax.nn.sigmoid(jnp.sum(x * gw, axis=-1, keepdims=True))

    y_scale = jax.nn.sigmoid(r_sel) * (1.0 - gate_of(x_sel))

    def emit(s, a, keep=None):
        row = pl.ds(pl.multiple_of(s * seg, seg), seg)
        x = x_sc[row, :].astype(_F32)
        gate = gate_of(x)
        mixed = gate * a + (1.0 - gate) * x
        if keep is not None:
            mixed = jnp.where(keep, mixed, 0.0)
        o_sc[row, :] = (o_sc[row, :].astype(_F32) + mixed).astype(_BF16)

    def ffn_block(n, live):
        gate = up = None
        for c in range(2):
            cols = slice(c * hd, (c + 1) * hd)
            rows = slice(c * hd // 2, (c + 1) * hd // 2)
            z = _dot(o_sc[S:, cols].astype(_F32)[:_TOPK], pltpu.bitcast(wg_sc[n, rows, :], _BF16))
            gate = z if c == 0 else z + gate
            yield
            z = _dot(o_sc[S:, cols].astype(_F32)[:_TOPK], pltpu.bitcast(wu_sc[n, rows, :], _BF16))
            up = z if c == 0 else z + up
            yield
        hidden = jnp.where(live, gate * jax.nn.sigmoid(gate) * up, 0.0)
        for c in range(2):
            cols = slice(c * hd, (c + 1) * hd)
            y_sc[:, cols] += _dot(hidden, pltpu.bitcast(wd_sc[n, :, cols], _BF16))
            yield

    def step(s, mem, ffn, n_early):
        src = pl.multiple_of(r0 + s * ts, 8)
        fresh = x_sc[pl.ds(src, ts), :].astype(_F32)
        lhs = jnp.concatenate([mem, fresh], axis=0).astype(_BF16)
        put = [pl.multiple_of(lax.rem(src + 8 * i, n_ring), 8) for i in range(ts // 8)]
        get = pl.multiple_of(lax.rem(s * seg, n_ring), seg)
        early = {(h, 0): _dot(lhs[:, :hd], weight(h // 2, h % 2, 0, 0, hd))
                 for h in range(n_early)}

        def skipped(h):
            return 8 if h < H - _GROUP else 0

        def settle():
            ring[0, spare, :] = o_sc[S:, 0:E].astype(_F32)[:8]
            yield

        side = {_EMIT_BY: [settle()]}
        count = [0]

        def proj(h, t):
            if (h, t) in early:
                y = _dot(lhs[:, hd:], weight(h // 2, h % 2, t, hd, D)) + early[h, t]
            else:
                y = _dot(lhs, weight(h // 2, h % 2, t))
            for i in range(ts // 8):
                ring[3 * h + t, pl.ds(put[i], 8), :] = y[M + 8 * i:M + 8 * i + 8]
            if t == 0:
                tok = ring[3 * h, pl.ds(get + skipped(h), seg - skipped(h)), :]
                out = jnp.concatenate([y[:M], tok], axis=0)
            else:
                tok = ring[3 * h + t, pl.ds(get, seg), :]
                out = jnp.concatenate([tok, y[:M]], axis=0).astype(_BF16), y[:M]
            for f in side.pop(count[0], []):
                next(f, None)
            count[0] += 1
            return out

        def probs(h, q, k):
            sc = lax.dot_general(q, k[0], (((1,), (1,)), ((), ())), preferred_element_type=_F32)
            sc = sc * scale + bias[skipped(h)]
            p = jnp.exp2(sc - jnp.max(sc, axis=-1, keepdims=True))
            return p, jnp.sum(p, axis=-1, keepdims=True)

        def mix(ps, vs):
            return [_dot(p, v[0]) * _recip(total) for (p, total), v in zip(ps, vs)]

        first_rows = {}

        def attend_first(h, k_mem, v_mem):
            z, top = {}, None
            k_tok = ring[3 * h + 1, pl.ds(get, 8), :]
            for b, k in enumerate((k_mem, k_tok)):
                q = ring[3 * h, pl.ds(get, 8), :] * scale
                for j in range(8):
                    w = jnp.sum(q * jnp.broadcast_to(k[j:j + 1], (8, E)), axis=-1, keepdims=True)
                    if b == 1 and j > 0:
                        w = w + edge[j]
                    z[b, j] = w
                    top = w if top is None else jnp.maximum(top, w)
                yield
            yield
            ring[3 * h + 1, spare, :] = jnp.broadcast_to(top, (8, E))
            num = den = None
            v_tok = ring[3 * h + 2, pl.ds(get, 8), :]
            for b, v in enumerate((v_mem, v_tok)):
                top = ring[3 * h + 1, spare, :]
                for j in range(8):
                    p = jnp.exp2(z[b, j] - top)
                    pv = p * jnp.broadcast_to(v[j:j + 1], (8, E))
                    num = pv if num is None else num + pv
                    den = p if den is None else den + p
                if b == 1:
                    first_rows[h] = num * _recip(den)
                yield

        acc = [None] * n_d

        def out_proj(g, blocks):
            rows = slice(g * _GROUP * E // 2, (g + 1) * _GROUP * E // 2)
            heads = jnp.concatenate([
                jnp.concatenate([z[:M], first_rows[h], z[M:]], axis=0) if skipped(h) else z
                for h, z in enumerate(o[g], g * _GROUP)], axis=1)
            for n in blocks:
                y = _dot(heads, pltpu.bitcast(wo_sc[n, rows, :], _BF16))
                acc[n] = y if acc[n] is None else y + acc[n]
                if n == _FFN_AT and g in _FFN_STAGES:
                    next(ffn, None)

        o = {}
        p_prev = v_prev = None
        for g in range(n_grp):
            heads = range(g * _GROUP, (g + 1) * _GROUP)
            qkv = {}
            for c, (t, h) in enumerate([(t, h) for t in range(3) for h in heads]):
                qkv[t, h] = proj(h, t)
                if g > 0 and c == _MIX_AT:
                    o[g - 1] = mix(p_prev, v_prev)
            v_prev = [qkv[2, h] for h in heads]
            p_prev = [probs(h, qkv[0, h], qkv[1, h]) for h in heads]
            for i, h in enumerate(heads):
                if skipped(h):
                    f = attend_first(h, qkv[1, h][1], qkv[2, h][1])
                    for d in range(5):
                        side.setdefault(count[0] + 3 * i + d, []).append(f)
            if g == n_grp - 1:
                for key in sorted(side):
                    for f in side[key]:
                        next(f, None)
            if g > 1:
                out_proj(g - 2, range(n_d))
        out_proj(n_grp - 2, range(n_d // 4))
        o[n_grp - 1] = mix(p_prev, v_prev)
        out_proj(n_grp - 2, range(n_d // 4, n_d))
        out_proj(n_grp - 1, range(n_d))
        res = jnp.concatenate(acc, axis=1)
        return res[:M], res[M:]

    def steps(i, mem):
        @pl.when(i < n_f)
        def _():
            for cp in ffn_copies(i):
                cp.wait()

        @pl.when(i + 1 < n_f)
        def _():
            for cp in ffn_copies(i + 1):
                cp.start()

        @pl.when(i == n_f)
        def _():
            y = y_sc[...] * y_scale
            for c, (base, off) in enumerate(picks):
                rows = o_sc[pl.ds(base, 16), :].astype(_F32)
                rows = jnp.where(row16 == off, rows + y[c:c + 1, :], rows)
                o_sc[pl.ds(base, 16), :] = rows.astype(_BF16)
            out_copy(0, _UNROLL * n_f - 1).start()

        ffn = ffn_block(jnp.minimum(i, n_f - 1) & 1, i < n_f)
        emit(jnp.maximum(_UNROLL * i - 1, 0), a_sc[...], i > 0)
        mem, a = step(_UNROLL * i, mem, ffn, 0)
        emit(_UNROLL * i, a)
        mem, a = step(_UNROLL * i + 1, mem, ffn, _EARLY)
        for _ in ffn:
            pass
        a_sc[...] = a

        @pl.when(i >= n_f)
        def _():
            out_copy(_UNROLL * i - 1, _UNROLL).start()

        return mem

    lax.fori_loop(0, n_seg // _UNROLL, steps, mem0_sc[...].astype(_F32))
    emit(n_seg - 1, a_sc[...])
    out_copy(n_seg - 1, 1).start()
    out_copy(0, n_seg).wait()


@functools.partial(jax.jit, static_argnames=("A_seg_len",))
def pallas_gated_mix__memory_aug_recurrent_mem_tr__moe_arch_mod__prompt_kernel(
    A_x: jax.Array,
    A_mem0: jax.Array,
    A_Wq: jax.Array,
    A_Wk: jax.Array,
    A_Wv: jax.Array,
    A_Wo: jax.Array,
    A_seg_len: int,
    B_x: jax.Array,
    B_w_r: jax.Array,
    B_w_gate: jax.Array,
    B_w_up: jax.Array,
    B_w_down: jax.Array,
    gate_w: jax.Array,
):
    del B_x
    B, S, D = A_x.shape
    M = A_mem0.shape[1]
    H, E = A_Wq.shape[1:]
    F = B_w_gate.shape[1]
    seg = int(A_seg_len)
    assert (B, S, D, M, H, E, seg) == (1, 2048, 1024, 8, 32, _LANES, _STEP_ROWS)
    assert F % _LANES == 0 and F // _LANES < S // seg // _UNROLL
    r0 = S - (S // seg) * (_STEP_ROWS - M)

    hbm = pl.BlockSpec(memory_space=pl.ANY)
    slabs = lambda w: w.reshape(D // 16, 16, H, E)
    out = pl.pallas_call(
        functools.partial(_kernel, seg=seg),
        out_shape=jax.ShapeDtypeStruct((S, D), A_x.dtype),
        in_specs=[hbm] * 11,
        out_specs=hbm,
        scratch_shapes=[
            pltpu.VMEM((S, D), _BF16),
            pltpu.VMEM((S + 2 * _TOPK, D), _BF16),
            pltpu.VMEM((seg, D), _F32),
            pltpu.VMEM((_TOPK, D), _F32),
            pltpu.VMEM((3 * H // 2, D // 16, 16, E), _U32),
            pltpu.VMEM((D // _LANES, H * E // 2, _LANES), _U32),
            pltpu.VMEM((3 * H, r0 + seg + 16, E), _F32),
            pltpu.VMEM((2, D // 2, _LANES), _U32),
            pltpu.VMEM((2, D // 2, _LANES), _U32),
            pltpu.VMEM((2, _LANES // 2, D), _U32),
            pltpu.VMEM((M, D), _BF16),
            pltpu.VMEM((D,), _BF16),
            pltpu.VMEM((D,), _BF16),
            pltpu.VMEM((7, r0 // 4, D // 2), _U32),
            pltpu.VMEM((3, 5, D // 4, E), _U32),
            pltpu.SemaphoreType.DMA((8,)),
            pltpu.SemaphoreType.DMA((1,)),
            pltpu.SemaphoreType.DMA((1,)),
            pltpu.SemaphoreType.DMA((2,)),
            pltpu.SemaphoreType.DMA((1,)),
        ],
        compiler_params=pltpu.CompilerParams(
            vmem_limit_bytes=112 * 1024 * 1024, disable_bounds_checks=True),
    )(
        A_x.reshape(S, D), A_mem0.reshape(M, D),
        slabs(A_Wq), slabs(A_Wk), slabs(A_Wv), A_Wo.reshape(H * E, D),
        B_w_r, gate_w, B_w_gate, B_w_up, B_w_down,
    )
    return out.reshape(B, S, D)
```

```python
import functools

import jax
import jax.numpy as jnp
from jax import lax
import jax.experimental.pallas as pl
import jax.experimental.pallas.tpu as pltpu

_F32 = jnp.float32
_BF16 = jnp.bfloat16
_U32 = jnp.uint32
_LANES = 128
_TOPK = 8
_MASKED = -1e9
_STEP_ROWS = 32
_GROUP = 4
_UNROLL = 4
_EARLY = 3
_PIECE = 32
_MIX_AT = 7
_FFN_AT = 3
_FFN_STAGES = (3, 4, 5)
_EMIT_BY = 7

_PLAN = ((2, ((1, 0), (3, 0))), (3, ((2, 0), (0, 0))), (4, ((1, 1), (0, -1))),
         (1, ((2, 1), (3, -1))), (0, ((0, 1), (3, 1))), (5, ((3, 1),)), (6, ((0, 1),)))
_RHS_SLOT = (0, None, 1, 2, None, 3, 4)


def _lhs_terms(a11, a12, a21, a22):
    return a11 + a22, a21 + a22, a11, a22, a11 + a12, a21 - a11, a12 - a22


def _rhs_terms(b11, b12, b21, b22):
    return b11 + b22, b12 - b22, b21 - b11, b11 + b12, b21 + b22


def _dot(a, b):
    return jnp.dot(a, b, preferred_element_type=_F32)


def _recip(x):
    return pltpu.reciprocal(x, approx=True)


def _kernel(
    x_hbm, mem0_hbm, wq_hbm, wk_hbm, wv_hbm, wo_hbm, wr_hbm, gw_hbm,
    wg_hbm, wu_hbm, wd_hbm,
    out_hbm,
    x_sc, o_sc, a_sc, y_sc, w_sc, wo_sc, ring, wg_sc, wu_sc, wd_sc,
    mem0_sc, wr_sc, gw_sc, xa_sc, wb_sc, h_sc, raw_sc,
    w_sem, x_sem, wo_sem, ffn_sem, out_sem,
    *, seg,
):
    S, D = x_sc.shape
    M = mem0_sc.shape[0]
    H = w_sc.shape[0] // 3
    E = _LANES
    L = M + seg
    n_seg = S // seg
    ts = _STEP_ROWS - M
    r0 = S - n_seg * ts
    hr, hd = r0 // 2, D // 2
    n_ring = r0 + seg
    spare = slice(n_ring, n_ring + 8)
    n_pair = H // 2
    n_d = D // _LANES
    n_f = wg_hbm.shape[1] // _LANES
    scale = float(E) ** -0.5 * 1.4426950408889634

    w_hbm = [w.bitcast(_U32) for w in (wq_hbm, wk_hbm, wv_hbm)]
    wo_hbm, wg_hbm, wu_hbm, wd_hbm = [
        w.bitcast(_U32) for w in (wo_hbm, wg_hbm, wu_hbm, wd_hbm)]

    def w_copy(j, t):
        j, t = j + t // 3, t % 3
        slot = (3 * j + t) & (raw_sc.shape[0] - 1)
        return pltpu.make_async_copy(
            w_hbm[t].at[:, j, :], raw_sc.at[slot, 0:D], w_sem.at[slot])

    def x_copy(i):
        rows = pl.ds(pl.multiple_of(i * r0, r0), r0)
        return pltpu.make_async_copy(x_hbm.at[rows], x_sc.at[rows], x_sem.at[0])

    def lane_block(n):
        return pl.ds(pl.multiple_of(n * _LANES, _LANES), _LANES)

    def wo_copy(n):
        return pltpu.make_async_copy(wo_hbm.at[:, lane_block(n)], wo_sc.at[n], wo_sem.at[0])

    def ffn_copies(lo, hi, sem):
        cols = pl.ds(lo * _LANES, (hi - lo) * _LANES)
        rows = pl.ds(lo * _LANES // 2, (hi - lo) * _LANES // 2)
        return [pltpu.make_async_copy(wg_hbm.at[:, cols], wg_sc.at[:, cols], sem),
                pltpu.make_async_copy(wu_hbm.at[:, cols], wu_sc.at[:, cols], sem),
                pltpu.make_async_copy(wd_hbm.at[rows], wd_sc.at[rows], sem)]

    ffn_rate = _UNROLL // 2
    ffn_head = ffn_copies(0, ffn_rate, ffn_sem.at[0])
    ffn_rest = ffn_copies(ffn_rate, n_f, ffn_sem.at[1])

    def out_copy(first, count):
        rows = pl.ds(first * seg, count * seg)
        return pltpu.make_async_copy(o_sc.at[rows], out_hbm.at[rows], out_sem.at[0])

    def split_heads(j, t):
        j, t = j + t // 3, t % 3
        slot = (3 * j + t) & (raw_sc.shape[0] - 1)
        for c in range(0, hd // 2, 8):
            hi = pltpu.bitcast(ring[2, spare, :], _U32)
            lo = hi >> 16
            blocks = []
            for r in (c, c + hd // 2):
                even = raw_sc[slot, pl.ds(2 * r, 8, stride=2), :]
                odd = raw_sc[slot, pl.ds(2 * r + 1, 8, stride=2), :]
                pair = (even & lo) | (odd << 16), (even >> 16) | (odd & hi)
                for p in range(2):
                    w_sc[3 * (2 * j + p) + t, r:r + 8, :] = pair[p]
                    blocks.append(pltpu.bitcast(pair[p], _BF16).astype(_F32))
            for i, z in enumerate(_rhs_terms(*blocks)):
                wb_sc[t, i, c:c + 8, :] = pltpu.bitcast(z.astype(_BF16), _U32)
            yield

    def weight(h, t, lo=0, hi=D):
        return pltpu.bitcast(w_sc[3 * h + t, lo // 2:hi // 2, :], _BF16)

    x_copy(0).start()
    w_copy(0, 0).start()
    small = [pltpu.make_async_copy(a, b, wo_sem.at[0])
             for a, b in ((mem0_hbm, mem0_sc), (wr_hbm, wr_sc), (gw_hbm, gw_sc))]
    for cp in small:
        cp.start()
    o_sc[...] = jnp.zeros(o_sc.shape, _BF16)
    a_sc[...] = jnp.zeros(a_sc.shape, _F32)
    y_sc[...] = jnp.zeros(y_sc.shape, _F32)
    ring[2, spare, :] = pltpu.bitcast(jnp.full((8, E), 0xFFFF0000, _U32), _F32)
    for cp in small:
        cp.wait()
    w_copy(0, 0).wait()
    w_copy(0, 1).start()
    for _ in split_heads(0, 0):
        pass
    x_copy(0).wait()
    w_copy(0, 2).start()

    wr = wr_sc[...].astype(_F32).reshape(1, D)
    gw = gw_sc[...].astype(_F32).reshape(1, D)

    n_tok = S // n_pair
    per_x = r0 // n_tok
    per_product = hr // _PIECE
    group = (lax.broadcasted_iota(jnp.int32, (S // _LANES, _LANES), 0) // 8 * _LANES
             + lax.broadcasted_iota(jnp.int32, (S // _LANES, _LANES), 1))

    def route(score, row):
        r = jnp.sum(x_sc[pl.ds(pl.multiple_of(row, 16), 16), :].astype(_F32) * wr,
                    axis=-1, keepdims=True)
        for c in range(2):
            piece = jnp.concatenate([r[8 * c:8 * c + 8]] * (S // _LANES // 8), axis=0)
            score = jnp.where(group == row // 8 + c, piece, score)
        return score

    def project(j, score, overlap, route_from=4):
        for t in range(3):
            side = overlap(j, t)
            for c, (k, outs) in enumerate(_PLAN):
                if k == 1:
                    w = weight(2 * j, t, 0, hd)
                elif k == 4:
                    w = weight(2 * j + 1, t, hd, D)
                else:
                    w = pltpu.bitcast(wb_sc[t, _RHS_SLOT[k]], _BF16)
                if overlap is overlap_first and t == 0 and k in (2, 3):
                    a = x_sc[0:hr, 0:hd] if k == 2 else x_sc[hr:r0, hd:D]
                else:
                    a = pltpu.bitcast(xa_sc[k], _BF16)
                m = _dot(a, w)
                for r in range(0, hr, _PIECE):
                    for block, sign in outs:
                        row = block // 2 * hr + r
                        dst = (3 * (2 * j + block % 2) + t, slice(row, row + _PIECE))
                        z = m[r:r + _PIECE]
                        if sign:
                            z = ring[dst] + z if sign > 0 else ring[dst] - z
                        ring[dst] = z
                    next(side, None)
                if c >= route_from:
                    part = 16 * ((len(_PLAN) - route_from) * t + c - route_from)
                    if part <= n_tok:
                        ring[0, spare, :] = score[:8]
                    if part < n_tok:
                        score = route(score, j * n_tok + part)
            for _ in side:
                pass
        return score

    def overlap_first(j, t):
        idle = 4 * per_product - 1
        if t == 0:
            for i in range(0, hr, 16):
                terms = _lhs_terms(*[x_sc[r + i:r + i + 16, c:c + hd].astype(_F32)
                                     for r in (0, hr) for c in (0, hd)])
                for k, z in enumerate(terms):
                    xa_sc[k, i // 2:i // 2 + 8, :] = pltpu.bitcast(z.astype(_BF16), _U32)
                if i % 48 != 32 and i < hr - 16:
                    idle -= 1
                    yield
        if t < 2:
            for _ in range(idle):
                yield
            for u in ((1,), (2, 3))[t]:
                w_copy(j, u).wait()
            for u in ((3, 4), (5, 6))[t]:
                w_copy(j, u).start()
            yield
        for c, _ in enumerate(split_heads(j, t + 1)):
            if c % 3 or t == 2:
                yield

    def overlap_middle(j, t):
        for _ in range(per_product):
            yield
        yield from split_heads(j, t + 1)

    def overlap_last(j, t):
        if t < 2:
            yield from overlap_middle(j, t)

    def phase1(j, score):
        for t in range(1, 4):
            w_copy(j, t).wait()

        @pl.when((j & (per_x - 1)) == 0)
        def _():
            x_copy(j // per_x).wait()

        score = project(j, score, overlap_middle)

        for u in range(7, 10):
            @pl.when(3 * j + u < 3 * n_pair)
            def _():
                w_copy(j, u).start()

        @pl.when(jnp.logical_and((j & (per_x - 1)) == 0, j + per_x < n_pair))
        def _():
            x_copy(j // per_x + 1).start()

        @pl.when(((j - 1) & 3) < 2)
        def _():
            wo_copy(((j - 1) >> 2) * 2 + ((j - 1) & 3)).start()

        return score

    score = project(0, jnp.zeros((S // _LANES, _LANES), _F32), overlap_first)
    for u in range(7, 10):
        w_copy(0, u).start()
    x_copy(1).start()
    score = lax.fori_loop(1, n_pair - 1, phase1, score)
    for cp in ffn_head:
        cp.start()
    for t in range(1, 3):
        w_copy(n_pair - 1, t).wait()
    score = project(n_pair - 1, score, overlap_last, route_from=0)

    score = score.astype(_BF16).astype(_F32)
    score = jnp.where(score != score, -jnp.inf, score)
    token = (group * 8 + lax.broadcasted_iota(jnp.int32, group.shape, 0) % 8).astype(_F32)
    picks = []
    row8 = lax.broadcasted_iota(jnp.int32, (8, 1), 0)
    row16 = lax.broadcasted_iota(jnp.int32, (16, 1), 0)
    r_sel = jnp.zeros((_TOPK, 1), _F32)
    x_sel = jnp.zeros((_TOPK, D), _F32)
    for c in range(_TOPK):
        best = jnp.max(jnp.max(score, axis=0, keepdims=True), axis=1, keepdims=True)
        first = jnp.where(score == best, token, float(S))
        first = jnp.min(jnp.min(first, axis=0, keepdims=True), axis=1, keepdims=True)
        taken = token == first
        score = jnp.where(taken, -jnp.inf, score)
        token = jnp.where(taken, float(S), token)
        idx = jnp.clip(first.astype(jnp.int32)[0, 0], 0, S - 1)
        base = pl.multiple_of((idx // 16) * 16, 16)
        rows = x_sc[pl.ds(base, 16), :].astype(_F32)
        picked = jnp.sum(jnp.where(row16 == idx - base, rows, 0.0), axis=0, keepdims=True)
        x_sel = jnp.where(row8 == c, picked, x_sel)
        r_sel = jnp.where(row8 == c, best, r_sel)
        picks.append((base, idx - base))
    o_sc[S:, :] = jnp.concatenate([x_sel, x_sel], axis=0).astype(_BF16)
    for cp in ffn_head:
        cp.wait()
    for cp in ffn_rest:
        cp.start()
    pltpu.make_async_copy(wo_sc, wo_sc, wo_sem.at[0]).wait()

    n_grp = H // _GROUP

    def skipped(h):
        return 8 if h < H - _GROUP else 0

    def mask_bias(skip):
        qi = lax.broadcasted_iota(jnp.int32, (L - skip, L), 0)
        ki = lax.broadcasted_iota(jnp.int32, (L - skip, L), 1)
        return jnp.where((qi < M) | (ki >= seg) | (ki <= qi - M + skip), 0.0, _MASKED)

    bias = {skip: mask_bias(skip) for skip in (0, 8)}
    edge = {j: jnp.where(row8 >= j, 0.0, _MASKED) for j in range(1, 8)}

    def gate_of(x):
        return jax.nn.sigmoid(jnp.sum(x * gw, axis=-1, keepdims=True))

    y_scale = jax.nn.sigmoid(r_sel) * (1.0 - gate_of(x_sel))

    def emit(s, a, keep=None):
        row = pl.ds(pl.multiple_of(s * seg, seg), seg)
        x = x_sc[row, :].astype(_F32)
        gate = gate_of(x)
        mixed = gate * a + (1.0 - gate) * x
        if keep is not None:
            mixed = jnp.where(keep, mixed, 0.0)
        o_sc[row, :] = (o_sc[row, :].astype(_F32) + mixed).astype(_BF16)

    def ffn_block(n):
        live = jnp.logical_and(n >= 0, n < n_f)
        n = jnp.clip(n, 0, n_f - 1)
        gate = up = None
        for c in range(2):
            cols = slice(c * hd, (c + 1) * hd)
            rows = slice(c * hd // 2, (c + 1) * hd // 2)
            z = _dot(o_sc[S:, cols].astype(_F32)[:_TOPK],
                     pltpu.bitcast(wg_sc[rows, lane_block(n)], _BF16))
            gate = z if c == 0 else z + gate
            yield
            z = _dot(o_sc[S:, cols].astype(_F32)[:_TOPK],
                     pltpu.bitcast(wu_sc[rows, lane_block(n)], _BF16))
            up = z if c == 0 else z + up
            yield
        hidden = jnp.where(live, gate * jax.nn.sigmoid(gate) * up, 0.0)
        rows = pl.ds(pl.multiple_of(n * (E // 2), E // 2), E // 2)
        for c in range(2):
            cols = slice(c * hd, (c + 1) * hd)
            y_sc[:, cols] += _dot(hidden, pltpu.bitcast(wd_sc[rows, cols], _BF16))
            yield

    def step(s, mem, ffn, n_early):
        src = pl.multiple_of(r0 + s * ts, 8)
        fresh = x_sc[pl.ds(src, ts), :].astype(_F32)
        h_sc[...] = pltpu.bitcast(jnp.concatenate([mem, fresh], axis=0).astype(_BF16), _U32)
        put = [pl.multiple_of(lax.rem(src + 8 * i, n_ring), 8) for i in range(ts // 8)]
        get = pl.multiple_of(lax.rem(s * seg, n_ring), seg)

        def partial_proj(h, t, lo, hi):
            return _dot(pltpu.bitcast(h_sc[:, lo:hi], _BF16), weight(h, t, lo, hi))

        early = {(h, 0): partial_proj(h, 0, 0, hd) for h in range(n_early)}

        def settle():
            ring[0, spare, :] = o_sc[S:, 0:E].astype(_F32)[:8]
            yield

        side = {_EMIT_BY: [settle()]}
        count = [0]

        def proj(h, t):
            if (h, t) in early:
                y = partial_proj(h, t, hd, D) + early[h, t]
            else:
                y = partial_proj(h, t, 0, D)
            for i in range(ts // 8):
                ring[3 * h + t, pl.ds(put[i], 8), :] = y[M + 8 * i:M + 8 * i + 8]
            if t == 0:
                tok = ring[3 * h, pl.ds(get + skipped(h), seg - skipped(h)), :]
                out = jnp.concatenate([y[:M], tok], axis=0)
            else:
                tok = ring[3 * h + t, pl.ds(get, seg), :]
                out = jnp.concatenate([tok, y[:M]], axis=0).astype(_BF16), y[:M]
            for f in side.pop(count[0], []):
                next(f, None)
            count[0] += 1
            return out

        def probs(h, q, k):
            sc = lax.dot_general(q, k[0], (((1,), (1,)), ((), ())), preferred_element_type=_F32)
            sc = sc * scale + bias[skipped(h)]
            p = jnp.exp2(sc - jnp.max(sc, axis=-1, keepdims=True))
            return p, jnp.sum(p, axis=-1, keepdims=True)

        def mix(ps, vs):
            return [_dot(p, v[0]) * _recip(total) for (p, total), v in zip(ps, vs)]

        first_rows = {}

        def attend_first(h, k_mem, v_mem):
            z, top = {}, None
            k_tok = ring[3 * h + 1, pl.ds(get, 8), :]
            for b, k in enumerate((k_mem, k_tok)):
                q = ring[3 * h, pl.ds(get, 8), :] * scale
                for j in range(8):
                    w = jnp.sum(q * jnp.broadcast_to(k[j:j + 1], (8, E)), axis=-1, keepdims=True)
                    if b == 1 and j > 0:
                        w = w + edge[j]
                    z[b, j] = w
                    top = w if top is None else jnp.maximum(top, w)
                yield
            yield
            ring[3 * h + 1, spare, :] = jnp.broadcast_to(top, (8, E))
            num = den = None
            v_tok = ring[3 * h + 2, pl.ds(get, 8), :]
            for b, v in enumerate((v_mem, v_tok)):
                top = ring[3 * h + 1, spare, :]
                for j in range(8):
                    p = jnp.exp2(z[b, j] - top)
                    pv = p * jnp.broadcast_to(v[j:j + 1], (8, E))
                    num = pv if num is None else num + pv
                    den = p if den is None else den + p
                if b == 1:
                    first_rows[h] = num * _recip(den)
                yield

        acc = [None] * n_d

        def out_proj(g, blocks):
            rows = slice(g * _GROUP * E // 2, (g + 1) * _GROUP * E // 2)
            heads = jnp.concatenate([
                jnp.concatenate([z[:M], first_rows[h], z[M:]], axis=0) if skipped(h) else z
                for h, z in enumerate(o[g], g * _GROUP)], axis=1)
            for n in blocks:
                y = _dot(heads, pltpu.bitcast(wo_sc[n, rows, :], _BF16))
                acc[n] = y if acc[n] is None else y + acc[n]
                if n == _FFN_AT and g in _FFN_STAGES:
                    next(ffn)

        o = {}
        p_prev = v_prev = None
        for g in range(n_grp):
            heads = range(g * _GROUP, (g + 1) * _GROUP)
            qkv = {}
            for c, (t, h) in enumerate([(t, h) for t in range(3) for h in heads]):
                qkv[t, h] = proj(h, t)
                if g > 0 and c == _MIX_AT:
                    o[g - 1] = mix(p_prev, v_prev)
            v_prev = [qkv[2, h] for h in heads]
            p_prev = [probs(h, qkv[0, h], qkv[1, h]) for h in heads]
            for i, h in enumerate(heads):
                if skipped(h):
                    f = attend_first(h, qkv[1, h][1], qkv[2, h][1])
                    for d in range(5):
                        side.setdefault(count[0] + 3 * i + d, []).append(f)
            if g == n_grp - 1:
                for key in sorted(side):
                    for f in side[key]:
                        next(f, None)
            if g > 1:
                out_proj(g - 2, range(n_d))
        out_proj(n_grp - 2, range(n_d // 4))
        o[n_grp - 1] = mix(p_prev, v_prev)
        out_proj(n_grp - 2, range(n_d // 4, n_d))
        out_proj(n_grp - 1, range(n_d))
        res = jnp.concatenate(acc, axis=1)
        return res[:M], res[M:]

    n_iter = n_seg // _UNROLL
    lead = n_iter - 1 - n_f // ffn_rate

    def steps(i, mem):
        @pl.when(jnp.logical_or(i == lead + 1, i == n_iter - 1))
        def _():
            @pl.when(i == lead + 1)
            def _():
                for cp in ffn_rest:
                    cp.wait()

            @pl.when(i == n_iter - 1)
            def _():
                y = y_sc[...] * y_scale
                for c, (base, off) in enumerate(picks):
                    rows = o_sc[pl.ds(base, 16), :].astype(_F32)
                    rows = jnp.where(row16 == off, rows + y[c:c + 1, :], rows)
                    o_sc[pl.ds(base, 16), :] = rows.astype(_BF16)
                out_copy(0, n_seg - _UNROLL - 1).start()

        a = a_sc[...]
        for u in range(_UNROLL):
            s = _UNROLL * i + u
            if u % 2 == 0:
                ffn = ffn_block((i - lead) * ffn_rate + u // 2)
            if u == 0:
                emit(jnp.maximum(s - 1, 0), a, i > 0)
            else:
                emit(s - 1, a)
            mem, a = step(s, mem, ffn, _EARLY if u else 0)
        a_sc[...] = a
        return mem

    lax.fori_loop(0, n_iter, steps, mem0_sc[...].astype(_F32))
    out_copy(n_seg - _UNROLL - 1, _UNROLL).start()
    emit(n_seg - 1, a_sc[...])
    out_copy(n_seg - 1, 1).start()
    out_copy(0, n_seg).wait()


@functools.partial(jax.jit, static_argnames=("A_seg_len",))
def pallas_gated_mix__memory_aug_recurrent_mem_tr__moe_arch_mod__prompt_kernel(
    A_x: jax.Array,
    A_mem0: jax.Array,
    A_Wq: jax.Array,
    A_Wk: jax.Array,
    A_Wv: jax.Array,
    A_Wo: jax.Array,
    A_seg_len: int,
    B_x: jax.Array,
    B_w_r: jax.Array,
    B_w_gate: jax.Array,
    B_w_up: jax.Array,
    B_w_down: jax.Array,
    gate_w: jax.Array,
):
    del B_x
    B, S, D = A_x.shape
    M = A_mem0.shape[1]
    H, E = A_Wq.shape[1:]
    F = B_w_gate.shape[1]
    seg = int(A_seg_len)
    assert (B, S, D, M, H, E, seg, F) == (1, 2048, 1024, 8, 32, _LANES, _STEP_ROWS, 3584)
    r0 = S - (S // seg) * (_STEP_ROWS - M)

    hbm = pl.BlockSpec(memory_space=pl.ANY)
    out = pl.pallas_call(
        functools.partial(_kernel, seg=seg),
        out_shape=jax.ShapeDtypeStruct((S, D), A_x.dtype),
        in_specs=[hbm] * 11,
        out_specs=hbm,
        scratch_shapes=[
            pltpu.VMEM((S, D), _BF16),
            pltpu.VMEM((S + 2 * _TOPK, D), _BF16),
            pltpu.VMEM((seg, D), _F32),
            pltpu.VMEM((_TOPK, D), _F32),
            pltpu.VMEM((3 * H, D // 2, E), _U32),
            pltpu.VMEM((D // _LANES, H * E // 2, _LANES), _U32),
            pltpu.VMEM((3 * H, r0 + seg + 16, E), _F32),
            pltpu.VMEM((D // 2, F), _U32),
            pltpu.VMEM((D // 2, F), _U32),
            pltpu.VMEM((F // 2, D), _U32),
            pltpu.VMEM((M, D), _BF16),
            pltpu.VMEM((D,), _BF16),
            pltpu.VMEM((D,), _BF16),
            pltpu.VMEM((7, r0 // 4, D // 2), _U32),
            pltpu.VMEM((3, 5, D // 4, E), _U32),
            pltpu.VMEM((_STEP_ROWS // 2, D), _U32),
            pltpu.VMEM((8, D + 8, E), _U32),
            pltpu.SemaphoreType.DMA((8,)),
            pltpu.SemaphoreType.DMA((1,)),
            pltpu.SemaphoreType.DMA((1,)),
            pltpu.SemaphoreType.DMA((2,)),
            pltpu.SemaphoreType.DMA((1,)),
        ],
        compiler_params=pltpu.CompilerParams(
            vmem_limit_bytes=112 * 1024 * 1024, disable_bounds_checks=True),
    )(
        A_x.reshape(S, D), A_mem0.reshape(M, D),
        A_Wq, A_Wk, A_Wv, A_Wo.reshape(H * E, D),
        B_w_r, gate_w, B_w_gate, B_w_up, B_w_down,
    )
    return out.reshape(B, S, D)
```

```python
import functools

import jax
import jax.numpy as jnp
from jax import lax
import jax.experimental.pallas as pl
import jax.experimental.pallas.tpu as pltpu

_F32 = jnp.float32
_BF16 = jnp.bfloat16
_U32 = jnp.uint32
_LANES = 128
_TOPK = 8
_LOG2E = 1.4426950408889634
_MASKED = -1e9 * _LOG2E
_STEP_ROWS = 32
_GROUP = 4
_UNROLL = 4
_EARLY = 3
_PIECE = 32
_MIX_AT = 7
_FFN_AT = 3
_FFN_STAGES = (3, 4, 5)
_EMIT_BY = 7


def _dot(a, b):
    return jnp.dot(a, b, preferred_element_type=_F32)


def _recip(x):
    return pltpu.reciprocal(x, approx=True)


def _kernel(
    x_hbm, mem0_hbm, wq_hbm, wk_hbm, wv_hbm, wo_hbm, wr_hbm, gw_hbm,
    wg_hbm, wu_hbm, wd_hbm,
    out_hbm,
    x_sc, o_sc, a_sc, y_sc, w_sc, wo_sc, ring, wg_sc, wu_sc, wd_sc,
    mem0_sc, wr_sc, gw_sc, h_sc, raw_sc,
    w_sem, x_sem, wo_sem, ffn_sem, out_sem,
    *, seg,
):
    S, D = x_sc.shape
    M = mem0_sc.shape[0]
    H = w_sc.shape[0] // 3
    E = _LANES
    L = M + seg
    n_seg = S // seg
    ts = _STEP_ROWS - M
    r0 = S - n_seg * ts
    hd = D // 2
    n_ring = r0 + seg
    spare = slice(n_ring, n_ring + 8)
    n_pair = H // 2
    n_d = D // _LANES
    n_f = wg_hbm.shape[1] // _LANES
    scale = float(E) ** -0.5 * _LOG2E

    w_hbm = [w.bitcast(_U32) for w in (wq_hbm, wk_hbm, wv_hbm)]
    wo_hbm, wg_hbm, wu_hbm, wd_hbm = [
        w.bitcast(_U32) for w in (wo_hbm, wg_hbm, wu_hbm, wd_hbm)]

    def w_copy(j, t):
        j, t = j + t // 3, t % 3
        slot = (3 * j + t) & (raw_sc.shape[0] - 1)
        return pltpu.make_async_copy(
            w_hbm[t].at[:, j, :], raw_sc.at[slot, 0:D], w_sem.at[slot])

    def x_copy(i):
        rows = pl.ds(pl.multiple_of(i * r0, r0), r0)
        return pltpu.make_async_copy(x_hbm.at[rows], x_sc.at[rows], x_sem.at[0])

    def lane_block(n):
        return pl.ds(pl.multiple_of(n * _LANES, _LANES), _LANES)

    def wo_copy(n):
        return pltpu.make_async_copy(wo_hbm.at[:, lane_block(n)], wo_sc.at[n], wo_sem.at[0])

    def ffn_copies(lo, hi, sem):
        cols = pl.ds(lo * _LANES, (hi - lo) * _LANES)
        rows = pl.ds(lo * _LANES // 2, (hi - lo) * _LANES // 2)
        return [pltpu.make_async_copy(wg_hbm.at[:, cols], wg_sc.at[:, cols], sem),
                pltpu.make_async_copy(wu_hbm.at[:, cols], wu_sc.at[:, cols], sem),
                pltpu.make_async_copy(wd_hbm.at[rows], wd_sc.at[rows], sem)]

    ffn_rate = _UNROLL // 2
    ffn_head = ffn_copies(0, ffn_rate, ffn_sem.at[0])
    ffn_rest = ffn_copies(ffn_rate, n_f, ffn_sem.at[1])

    def out_copy(first, count):
        rows = pl.ds(first * seg, count * seg)
        return pltpu.make_async_copy(o_sc.at[rows], out_hbm.at[rows], out_sem.at[0])

    def split_heads(j, t):
        j, t = j + t // 3, t % 3
        slot = (3 * j + t) & (raw_sc.shape[0] - 1)
        for c in range(0, hd, 32):
            hi = pltpu.bitcast(ring[2, spare, :], _U32)
            lo = hi >> 16
            for r in range(c, c + 32, 8):
                even = raw_sc[slot, pl.ds(2 * r, 8, stride=2), :]
                odd = raw_sc[slot, pl.ds(2 * r + 1, 8, stride=2), :]
                w_sc[6 * j + t, r:r + 8, :] = (even & lo) | (odd << 16)
                w_sc[6 * j + 3 + t, r:r + 8, :] = (even >> 16) | (odd & hi)
            yield

    def weight(h, t, lo=0, hi=D):
        return pltpu.bitcast(w_sc[3 * h + t, lo // 2:hi // 2, :], _BF16)

    x_copy(0).start()
    w_copy(0, 0).start()
    small = [pltpu.make_async_copy(a, b, wo_sem.at[0])
             for a, b in ((mem0_hbm, mem0_sc), (wr_hbm, wr_sc), (gw_hbm, gw_sc))]
    for cp in small:
        cp.start()
    o_sc[...] = jnp.zeros(o_sc.shape, _BF16)
    a_sc[...] = jnp.zeros(a_sc.shape, _F32)
    y_sc[...] = jnp.zeros(y_sc.shape, _F32)
    ring[2, spare, :] = pltpu.bitcast(jnp.full((8, E), 0xFFFF0000, _U32), _F32)
    for cp in small:
        cp.wait()
    w_copy(0, 0).wait()
    w_copy(0, 1).start()
    for _ in split_heads(0, 0):
        pass
    x_copy(0).wait()
    w_copy(0, 2).start()

    wr = wr_sc[...].astype(_F32).reshape(1, D)
    gw = gw_sc[...].astype(_F32).reshape(1, D)

    n_tok = S // n_pair
    per_x = r0 // n_tok
    n_piece = r0 // _PIECE
    group = (lax.broadcasted_iota(jnp.int32, (S // _LANES, _LANES), 0) // 8 * _LANES
             + lax.broadcasted_iota(jnp.int32, (S // _LANES, _LANES), 1))

    def route(score, row):
        r = jnp.sum(x_sc[pl.ds(pl.multiple_of(row, 16), 16), :].astype(_F32) * wr,
                    axis=-1, keepdims=True)
        for c in range(2):
            piece = jnp.concatenate([r[8 * c:8 * c + 8]] * (S // _LANES // 8), axis=0)
            score = jnp.where(group == row // 8 + c, piece, score)
        return score

    def project(j, score, overlap, route_every):
        routed = 0
        for t in range(3):
            side = overlap(j, t)
            ws = [weight(2 * j + p, t) for p in range(2)]
            for p in range(2):
                y = _dot(x_sc[0:r0, :], ws[p])
                for c in range(n_piece):
                    rows = slice(c * _PIECE, (c + 1) * _PIECE)
                    ring[3 * (2 * j + p) + t, rows, :] = y[rows]
                    next(side, None)
                    if c % route_every == 0 and routed <= n_tok:
                        ring[0, spare, :] = score[:8]
                        if routed < n_tok:
                            score = route(score, j * n_tok + routed)
                        routed += 16
            for _ in side:
                pass
        assert routed > n_tok
        return score

    def overlap_first(j, t):
        if t < 2:
            for _ in range(n_piece - 1):
                yield
            for u in ((1,), (2, 3))[t]:
                w_copy(j, u).wait()
            for u in ((3, 4), (5, 6))[t]:
                w_copy(j, u).start()
            yield
        yield from split_heads(j, t + 1)

    def overlap_middle(j, t):
        yield from split_heads(j, t + 1)

    def overlap_last(j, t):
        if t < 2:
            yield from split_heads(j, t + 1)

    def phase1(j, score):
        for t in range(1, 4):
            w_copy(j, t).wait()

        @pl.when((j & (per_x - 1)) == 0)
        def _():
            x_copy(j // per_x).wait()

        score = project(j, score, overlap_middle, 8)

        for u in range(7, 10):
            @pl.when(3 * j + u < 3 * n_pair)
            def _():
                w_copy(j, u).start()

        @pl.when(jnp.logical_and((j & (per_x - 1)) == 0, j + per_x < n_pair))
        def _():
            x_copy(j // per_x + 1).start()

        @pl.when(((j - 1) & 3) < 2)
        def _():
            wo_copy(((j - 1) >> 2) * 2 + ((j - 1) & 3)).start()

        return score

    score = project(0, jnp.zeros((S // _LANES, _LANES), _F32), overlap_first, 8)
    for u in range(7, 10):
        w_copy(0, u).start()
    x_copy(1).start()
    score = lax.fori_loop(1, n_pair - 1, phase1, score)
    for cp in ffn_head:
        cp.start()
    for t in range(1, 3):
        w_copy(n_pair - 1, t).wait()
    score = project(n_pair - 1, score, overlap_last, 3)

    score = score.astype(_BF16).astype(_F32)
    score = jnp.where(score != score, -jnp.inf, score)
    token = (group * 8 + lax.broadcasted_iota(jnp.int32, group.shape, 0) % 8).astype(_F32)
    picks = []
    row8 = lax.broadcasted_iota(jnp.int32, (8, 1), 0)
    row16 = lax.broadcasted_iota(jnp.int32, (16, 1), 0)
    r_sel = jnp.zeros((_TOPK, 1), _F32)
    x_sel = jnp.zeros((_TOPK, D), _F32)
    for c in range(_TOPK):
        best = jnp.max(jnp.max(score, axis=0, keepdims=True), axis=1, keepdims=True)
        first = jnp.where(score == best, token, float(S))
        first = jnp.min(jnp.min(first, axis=0, keepdims=True), axis=1, keepdims=True)
        taken = token == first
        score = jnp.where(taken, -jnp.inf, score)
        token = jnp.where(taken, float(S), token)
        idx = jnp.clip(first.astype(jnp.int32)[0, 0], 0, S - 1)
        base = pl.multiple_of((idx // 16) * 16, 16)
        rows = x_sc[pl.ds(base, 16), :].astype(_F32)
        picked = jnp.sum(jnp.where(row16 == idx - base, rows, 0.0), axis=0, keepdims=True)
        x_sel = jnp.where(row8 == c, picked, x_sel)
        r_sel = jnp.where(row8 == c, best, r_sel)
        picks.append((base, idx - base))
    o_sc[S:, :] = jnp.concatenate([x_sel, x_sel], axis=0).astype(_BF16)
    for cp in ffn_head:
        cp.wait()
    for cp in ffn_rest:
        cp.start()
    pltpu.make_async_copy(wo_sc, wo_sc, wo_sem.at[0]).wait()

    n_grp = H // _GROUP

    def skipped(h):
        return 8 if h < H - _GROUP else 0

    def mask_cap(skip):
        qi = lax.broadcasted_iota(jnp.int32, (L - skip, L), 0)
        ki = lax.broadcasted_iota(jnp.int32, (L - skip, L), 1)
        return jnp.where((qi < M) | (ki >= seg) | (ki <= qi - M + skip), jnp.inf, _MASKED)

    cap = {skip: mask_cap(skip) for skip in (0, 8)}
    edge = {j: jnp.where(row8 >= j, jnp.inf, _MASKED) for j in range(1, 8)}

    def gate_of(x):
        return jax.nn.sigmoid(jnp.sum(x * gw, axis=-1, keepdims=True))

    y_scale = jax.nn.sigmoid(r_sel) * (1.0 - gate_of(x_sel))

    def emit(s, a, keep=None):
        row = pl.ds(pl.multiple_of(s * seg, seg), seg)
        x = x_sc[row, :].astype(_F32)
        gate = gate_of(x)
        mixed = gate * a + (1.0 - gate) * x
        if keep is not None:
            mixed = jnp.where(keep, mixed, 0.0)
        o_sc[row, :] = (o_sc[row, :].astype(_F32) + mixed).astype(_BF16)

    def ffn_block(n):
        live = jnp.logical_and(n >= 0, n < n_f)
        n = jnp.clip(n, 0, n_f - 1)
        gate = up = None
        for c in range(2):
            cols = slice(c * hd, (c + 1) * hd)
            rows = slice(c * hd // 2, (c + 1) * hd // 2)
            z = _dot(o_sc[S:, cols].astype(_F32)[:_TOPK],
                     pltpu.bitcast(wg_sc[rows, lane_block(n)], _BF16))
            gate = z if c == 0 else z + gate
            yield
            z = _dot(o_sc[S:, cols].astype(_F32)[:_TOPK],
                     pltpu.bitcast(wu_sc[rows, lane_block(n)], _BF16))
            up = z if c == 0 else z + up
            yield
        hidden = jnp.where(live, gate * jax.nn.sigmoid(gate) * up, 0.0)
        rows = pl.ds(pl.multiple_of(n * (E // 2), E // 2), E // 2)
        for c in range(2):
            cols = slice(c * hd, (c + 1) * hd)
            y_sc[:, cols] += _dot(hidden, pltpu.bitcast(wd_sc[rows, cols], _BF16))
            yield

    def step(s, mem, ffn, n_early):
        src = pl.multiple_of(r0 + s * ts, 8)
        fresh = x_sc[pl.ds(src, ts), :].astype(_F32)
        h_sc[...] = pltpu.bitcast(jnp.concatenate([mem, fresh], axis=0).astype(_BF16), _U32)
        put = [pl.multiple_of(lax.rem(src + 8 * i, n_ring), 8) for i in range(ts // 8)]
        get = pl.multiple_of(lax.rem(s * seg, n_ring), seg)

        def partial_proj(h, t, lo, hi):
            return _dot(pltpu.bitcast(h_sc[:, lo:hi], _BF16), weight(h, t, lo, hi))

        early = {(h, 0): partial_proj(h, 0, 0, hd) for h in range(n_early)}

        def settle():
            ring[0, spare, :] = o_sc[S:, 0:E].astype(_F32)[:8]
            yield

        side = {_EMIT_BY: [settle()]}
        count = [0]

        def proj(h, t):
            if (h, t) in early:
                y = partial_proj(h, t, hd, D) + early[h, t]
            else:
                y = partial_proj(h, t, 0, D)
            for i in range(ts // 8):
                ring[3 * h + t, pl.ds(put[i], 8), :] = y[M + 8 * i:M + 8 * i + 8]
            if t == 0:
                tok = ring[3 * h, pl.ds(get + skipped(h), seg - skipped(h)), :]
                out = jnp.concatenate([y[:M], tok], axis=0)
            else:
                tok = ring[3 * h + t, pl.ds(get, seg), :]
                out = jnp.concatenate([tok, y[:M]], axis=0).astype(_BF16), y[:M]
            for f in side.pop(count[0], []):
                next(f, None)
            count[0] += 1
            return out

        def probs(h, q, k):
            sc = lax.dot_general(q, k[0], (((1,), (1,)), ((), ())), preferred_element_type=_F32)
            sc = jnp.minimum(sc * scale, cap[skipped(h)])
            p = jnp.exp2(sc - jnp.max(sc, axis=-1, keepdims=True))
            return p, jnp.sum(p, axis=-1, keepdims=True)

        def mix(ps, vs):
            return [_dot(p, v[0]) * _recip(total) for (p, total), v in zip(ps, vs)]

        first_rows = {}

        def attend_first(h, k_mem, v_mem):
            z, top = {}, None
            k_tok = ring[3 * h + 1, pl.ds(get, 8), :]
            for b, k in enumerate((k_mem, k_tok)):
                q = ring[3 * h, pl.ds(get, 8), :] * scale
                for j in range(8):
                    w = jnp.sum(q * jnp.broadcast_to(k[j:j + 1], (8, E)), axis=-1, keepdims=True)
                    if b == 1 and j > 0:
                        w = jnp.minimum(w, edge[j])
                    z[b, j] = w
                    top = w if top is None else jnp.maximum(top, w)
                yield
            yield
            ring[3 * h + 1, spare, :] = jnp.broadcast_to(top, (8, E))
            num = den = None
            v_tok = ring[3 * h + 2, pl.ds(get, 8), :]
            for b, v in enumerate((v_mem, v_tok)):
                top = ring[3 * h + 1, spare, :]
                for j in range(8):
                    p = jnp.exp2(z[b, j] - top)
                    pv = p * jnp.broadcast_to(v[j:j + 1], (8, E))
                    num = pv if num is None else num + pv
                    den = p if den is None else den + p
                if b == 1:
                    first_rows[h] = num * _recip(den)
                yield

        acc = [None] * n_d

        def out_proj(g, blocks):
            rows = slice(g * _GROUP * E // 2, (g + 1) * _GROUP * E // 2)
            heads = jnp.concatenate([
                jnp.concatenate([z[:M], first_rows[h], z[M:]], axis=0) if skipped(h) else z
                for h, z in enumerate(o[g], g * _GROUP)], axis=1)
            for n in blocks:
                y = _dot(heads, pltpu.bitcast(wo_sc[n, rows, :], _BF16))
                acc[n] = y if acc[n] is None else y + acc[n]
                if n == _FFN_AT and g in _FFN_STAGES:
                    next(ffn)

        o = {}
        p_prev = v_prev = None
        for g in range(n_grp):
            heads = range(g * _GROUP, (g + 1) * _GROUP)
            qkv = {}
            for c, (t, h) in enumerate([(t, h) for t in range(3) for h in heads]):
                qkv[t, h] = proj(h, t)
                if g > 0 and c == _MIX_AT:
                    o[g - 1] = mix(p_prev, v_prev)
            v_prev = [qkv[2, h] for h in heads]
            p_prev = [probs(h, qkv[0, h], qkv[1, h]) for h in heads]
            for i, h in enumerate(heads):
                if skipped(h):
                    f = attend_first(h, qkv[1, h][1], qkv[2, h][1])
                    for d in range(5):
                        side.setdefault(count[0] + 3 * i + d, []).append(f)
            if g == n_grp - 1:
                for key in sorted(side):
                    for f in side[key]:
                        next(f, None)
            if g > 1:
                out_proj(g - 2, range(n_d))
        out_proj(n_grp - 2, range(n_d // 4))
        o[n_grp - 1] = mix(p_prev, v_prev)
        out_proj(n_grp - 2, range(n_d // 4, n_d))
        out_proj(n_grp - 1, range(n_d))
        res = jnp.concatenate(acc, axis=1)
        return res[:M], res[M:]

    n_iter = n_seg // _UNROLL
    lead = n_iter - 1 - n_f // ffn_rate

    def steps(i, mem):
        @pl.when(jnp.logical_or(i == lead + 1, i == n_iter - 1))
        def _():
            @pl.when(i == lead + 1)
            def _():
                for cp in ffn_rest:
                    cp.wait()

            @pl.when(i == n_iter - 1)
            def _():
                y = y_sc[...] * y_scale
                for c, (base, off) in enumerate(picks):
                    rows = o_sc[pl.ds(base, 16), :].astype(_F32)
                    rows = jnp.where(row16 == off, rows + y[c:c + 1, :], rows)
                    o_sc[pl.ds(base, 16), :] = rows.astype(_BF16)
                out_copy(0, n_seg - _UNROLL - 1).start()

        a = a_sc[...]
        for u in range(_UNROLL):
            s = _UNROLL * i + u
            if u % 2 == 0:
                ffn = ffn_block((i - lead) * ffn_rate + u // 2)
            if u == 0:
                emit(jnp.maximum(s - 1, 0), a, i > 0)
            else:
                emit(s - 1, a)
            mem, a = step(s, mem, ffn, _EARLY if u else 0)
        a_sc[...] = a
        return mem

    lax.fori_loop(0, n_iter, steps, mem0_sc[...].astype(_F32))
    out_copy(n_seg - _UNROLL - 1, _UNROLL).start()
    emit(n_seg - 1, a_sc[...])
    out_copy(n_seg - 1, 1).start()
    out_copy(0, n_seg).wait()


@functools.partial(jax.jit, static_argnames=("A_seg_len",))
def pallas_gated_mix__memory_aug_recurrent_mem_tr__moe_arch_mod__prompt_kernel(
    A_x: jax.Array,
    A_mem0: jax.Array,
    A_Wq: jax.Array,
    A_Wk: jax.Array,
    A_Wv: jax.Array,
    A_Wo: jax.Array,
    A_seg_len: int,
    B_x: jax.Array,
    B_w_r: jax.Array,
    B_w_gate: jax.Array,
    B_w_up: jax.Array,
    B_w_down: jax.Array,
    gate_w: jax.Array,
):
    del B_x
    B, S, D = A_x.shape
    M = A_mem0.shape[1]
    H, E = A_Wq.shape[1:]
    F = B_w_gate.shape[1]
    seg = int(A_seg_len)
    assert (B, S, D, M, H, E, seg, F) == (1, 2048, 1024, 8, 32, _LANES, _STEP_ROWS, 3584)
    r0 = S - (S // seg) * (_STEP_ROWS - M)

    hbm = pl.BlockSpec(memory_space=pl.ANY)
    out = pl.pallas_call(
        functools.partial(_kernel, seg=seg),
        out_shape=jax.ShapeDtypeStruct((S, D), A_x.dtype),
        in_specs=[hbm] * 11,
        out_specs=hbm,
        scratch_shapes=[
            pltpu.VMEM((S, D), _BF16),
            pltpu.VMEM((S + 2 * _TOPK, D), _BF16),
            pltpu.VMEM((seg, D), _F32),
            pltpu.VMEM((_TOPK, D), _F32),
            pltpu.VMEM((3 * H, D // 2, E), _U32),
            pltpu.VMEM((D // _LANES, H * E // 2, _LANES), _U32),
            pltpu.VMEM((3 * H, r0 + seg + 16, E), _F32),
            pltpu.VMEM((D // 2, F), _U32),
            pltpu.VMEM((D // 2, F), _U32),
            pltpu.VMEM((F // 2, D), _U32),
            pltpu.VMEM((M, D), _BF16),
            pltpu.VMEM((D,), _BF16),
            pltpu.VMEM((D,), _BF16),
            pltpu.VMEM((_STEP_ROWS // 2, D), _U32),
            pltpu.VMEM((8, D + 8, E), _U32),
            pltpu.SemaphoreType.DMA((8,)),
            pltpu.SemaphoreType.DMA((1,)),
            pltpu.SemaphoreType.DMA((1,)),
            pltpu.SemaphoreType.DMA((2,)),
            pltpu.SemaphoreType.DMA((1,)),
        ],
        compiler_params=pltpu.CompilerParams(
            vmem_limit_bytes=112 * 1024 * 1024, disable_bounds_checks=True),
    )(
        A_x.reshape(S, D), A_mem0.reshape(M, D),
        A_Wq, A_Wk, A_Wv, A_Wo.reshape(H * E, D),
        B_w_r, gate_w, B_w_gate, B_w_up, B_w_down,
    )
    return out.reshape(B, S, D)
```
